```python
import jax
import jax.numpy as jnp

def _softmax(x, axis=-1):
    return jax.nn.softmax(x, axis=axis)
def _gelu(x):
    return jax.nn.gelu(x, approximate=True)
def _silu(x):
    return jax.nn.silu(x)
def _sigmoid(x):
    return jax.nn.sigmoid(x)
def _layernorm(x, axis=-1, eps=1e-5):
    m = jnp.mean(x, axis=axis, keepdims=True)
    v = jnp.var(x, axis=axis, keepdims=True)
    return (x - m) / jnp.sqrt(v + eps)
def _scatter_add(tgt, idx, src, axis=0):
    return tgt.at[idx].add(src)
def _segment_sum(src, seg, n):
    return jax.ops.segment_sum(src, seg, n)
class _Rng:
    def __init__(self, key):
        self._k = key
    def _next(self):
        self._k, sub = jax.random.split(self._k)
        return sub
    def normal(self, shape):
        return jax.random.normal(self._next(), shape, dtype=jnp.bfloat16)
    def randint(self, lo, hi, shape):
        return jax.random.randint(self._next(), shape, lo, hi, dtype=jnp.int32)
    def uniform(self, shape, lo=0.0, hi=1.0):
        return jax.random.uniform(self._next(), shape, jnp.bfloat16, lo, hi)
    def permutation(self, n):
        return jax.random.permutation(self._next(), n)


kernel_name = 'gated_mix__sliding_block_cached__moe_arch_mod__decode'

def setup_inputs():
    _rng = _Rng(jax.random.key(int.from_bytes(__import__("os").urandom(4), "little")))
    _w = (lambda a: (lambda t: t.astype(jnp.bfloat16) if jnp.issubdtype(t.dtype, jnp.floating) else t)(jnp.asarray(a)))
    def _A_setup():
        B, Sq, D = 1, 1, 640
        Hq, Hkv, Sk, Dh = 32, 32, 32768, 192
        assert Hq % Hkv == 0, (Hq, Hkv)
        return {
            "x": _w((lambda *s: _rng.normal(s) * 0.05)(B, Sq, D)),
            "k_cache": _w((lambda *s: _rng.normal(s) * 0.05)(B, Hkv, Sk, Dh)),
            "v_cache": _w((lambda *s: _rng.normal(s) * 0.05)(B, Hkv, Sk, Dh)),
            "wq": _w((lambda *s: _rng.normal(s) * 0.05)(D, Hq * Dh) * (D ** -0.5)),
            "wo": _w((lambda *s: _rng.normal(s) * 0.05)(Hq * Dh, D) * ((Hq * Dh) ** -0.5)),
        }
    _A_in = _A_setup()

    def _B_setup():
        B, S, D, F, C = 1, 1, 640, 1536, 1
        return {
            "x": _w((lambda *s: _rng.normal(s) * 0.05)(B, S, D)),
            "w_r": _w((lambda *s: _rng.normal(s) * 0.05)(D)),
            "w_gate": _w((lambda *s: _rng.normal(s) * 0.05)(D, F)),
            "w_up": _w((lambda *s: _rng.normal(s) * 0.05)(D, F)),
            "w_down": _w((lambda *s: _rng.normal(s) * 0.05)(F, D)),
        }
    _B_in = _B_setup()

    return {
        "A_x": _A_in["x"],
        "A_k_cache": _A_in["k_cache"],
        "A_v_cache": _A_in["v_cache"],
        "A_wq": _A_in["wq"],
        "A_wo": _A_in["wo"],
        "B_x": _B_in["x"],
        "B_w_r": _B_in["w_r"],
        "B_w_gate": _B_in["w_gate"],
        "B_w_up": _B_in["w_up"],
        "B_w_down": _B_in["w_down"],
        "gate_w": _w((lambda *s: _rng.normal(s) * 0.05)(640)),
    }

def reference(A_x, A_k_cache, A_v_cache, A_wq, A_wo, B_x, B_w_r, B_w_gate, B_w_up, B_w_down, gate_w):
    def _A_ref(x, k_cache, v_cache, wq, wo):
        B, Sq, D = x.shape
        Hq, Dh = 32, 192
        Hkv, Sk = k_cache.shape[1], k_cache.shape[2]
        W = min(4096, max(256, Sk // 4))
        rep = Hq // Hkv
        q = (lambda x, *d: x.transpose(*d))((x @ wq).reshape(B, Sq, Hq, Dh), 0, 2, 1, 3)
        k = jnp.repeat(k_cache[:, :, Sk - W:, :], rep, axis=1)
        v = jnp.repeat(v_cache[:, :, Sk - W:, :], rep, axis=1)
        scores = jnp.einsum("bhqd,bhkd->bhqk", q, k) * (Dh ** -0.5)
        p = _softmax(scores, axis=-1)
        o = jnp.einsum("bhqk,bhkd->bhqd", p, v)
        return (lambda x, *d: x.transpose(*d))(o, 0, 2, 1, 3).reshape(B, Sq, Hq * Dh) @ wo

    def _B_ref(x, w_r, w_gate, w_up, w_down):
        B, S, D = x.shape
        C = 1
        r = x @ w_r
        idx = jnp.argsort(-r, axis=-1)[:, :C]
        idx_e = jnp.repeat(idx.reshape(B, C, 1), D, axis=2)
        x_sel = jnp.take_along_axis(x, idx_e, axis=1)
        g = _silu(x_sel @ w_gate)
        u = x_sel @ w_up
        y = (g * u) @ w_down
        r_sel = _sigmoid(jnp.take_along_axis(r, idx, axis=1))
        y = y * r_sel.reshape(B, C, 1)
        b_off = (jnp.arange(B) * S).reshape(B, 1)
        flat_idx = (idx + b_off).reshape(B * C)
        zero = (x * 0.0).reshape(B * S, D)
        upd = _scatter_add(zero, flat_idx, y.reshape(B * C, D), axis=0)
        return x + upd.reshape(B, S, D)

    x = A_x
    g = _sigmoid((x * gate_w).sum(-1, keepdims=True))
    a = _A_ref(x, A_k_cache, A_v_cache, A_wq, A_wo)
    b = _B_ref(x, B_w_r, B_w_gate, B_w_up, B_w_down)
    return g * a + (1 - g) * b
```

```python
import contextlib

import jax
import jax.numpy as jnp
import jax.experimental.pallas as pl
import jax.experimental.pallas.tpu as pltpu

H, DH, SK, D, F = 32, 192, 32768, 640, 1536
W = min(4096, max(256, SK // 4))
BASE = SK - W
M = 8
KC = 512
NC = W // KC
RING = 16
HALF = 5
STEPS = 2 * HALF
f32 = jnp.float32
bf16 = jnp.bfloat16


def make(LOOK=10, GAP=20, GAP_P=30, GAP0=20, PRE0=20, TAIL=(8, 8, 8, 8, 8, 4, 2, 2), LAST_AT=8, LAST_GAP=20,
         scopes=False, compute=True):
    N_P, N_Q = 16, 3
    J0 = N_P + N_Q
    N_IT = J0 + H
    assert 1 + HALF * N_IT == H * NC
    wd_main = 112
    wd_last = F // 8 - wd_main - sum(TAIL)
    scope = (lambda n: jax.named_scope("T_" + n)) if scopes else (lambda n: contextlib.nullcontext())

    def mult(i, n):
        return i if isinstance(i, int) else pl.multiple_of(i, n)

    def kernel(x_hbm, kT, vT, wq, wo, wr_hbm, wg, wu, wd, gw_hbm, out_ref,
               x_v, wr_v, gw_v, wq_b, k_b, v_b, wo_b, wg_b, wu_b, wd_b,
               q_s, s_s, a_s, y_s, h_s, kv_sem, w_sem, s_sem, e_sem):
        def kv(which, t):
            h, c = t >> 3, mult((t & (NC - 1)) * KC, KC)
            src = (kT, vT)[which].at[0, h, :, pl.ds(BASE + c, KC)]
            dst = (k_b, v_b)[which].at[h & (RING - 1), :, pl.ds(c, KC)]
            return pltpu.make_async_copy(src, dst, kv_sem.at[which, t & 7])

        def wcopy(src, dst, r, nr, c, nc, sem):
            rows, cols = pl.ds(mult(r * 8, 8), nr * 8), pl.ds(c, nc)
            return pltpu.make_async_copy(src.at[rows, cols], dst.at[rows, cols], sem)

        streams = [(wq, wq_b, 0, N_P, 5, 512, 0), (wo, wo_b, J0 - 1, H, DH // 8, D, 1),
                   (wg, wg_b, N_P, 10, 8, 512, 0), (wu, wu_b, N_P + 10, 10, 8, 512, 0),
                   (wd, wd_b, N_P + 20, 14, 8, D, 0)]

        def active(it):
            return [s for s in streams if s[2] <= it < s[2] + s[3]]

        def w_pieces(rep, it):
            out = []
            for src, dst, i0, _, n, wc, k in active(rep):
                rc = [(r, c) for r in range(n) for c in range(0, src.shape[1], wc)]
                out += [((i + 0.5) / len(rc), k, (src, dst, (it - i0) * n + r, 1, c, wc, w_sem.at[k, it & 1]))
                        for i, (r, c) in enumerate(rc)]
            return [p[2] for p in sorted(out, key=lambda p: p[:2])]

        def w_wait(rep, it):
            for src, dst, i0, _, n, _, k in active(rep):
                wcopy(src, dst, (it - i0) * n, n, 0, src.shape[1], w_sem.at[k, it & 1]).wait()

        small = [pltpu.make_async_copy(x_hbm, x_v, s_sem.at[0]),
                 pltpu.make_async_copy(gw_hbm, gw_v, s_sem.at[1]),
                 pltpu.make_async_copy(wr_hbm, wr_v, s_sem.at[2])]

        def piece(it, s):
            di, s = divmod(s, STEPS)
            return s // HALF, 1 + HALF * (it + di) + s % HALF

        def xm():
            return jnp.broadcast_to(x_v[0], (2 * M, D))

        def q_block(b):
            c = mult(b * 2 * DH, 2 * DH)
            q = jnp.dot(xm(), wq_b[:, pl.ds(c, 2 * DH)], preferred_element_type=f32)[:M]
            q_s[2 * b] = q[:, :DH]
            q_s[2 * b + 1] = q[:, DH:]

        def gu_block(b):
            for i in range(2):
                c = pl.ds(mult(b * 256 + i * 128, 128), 128)
                g = jnp.dot(xm(), wg_b[:, c], preferred_element_type=f32)[0:1]
                u = jnp.dot(xm(), wu_b[:, c], preferred_element_type=f32)[0:1]
                h_s[c, :] = jnp.broadcast_to(jax.nn.silu(g) * u, (128, 128)).T

        def rows_dot(acc, w_ref, r0, col):
            for r in range(0, col.shape[0], 16):
                wf = w_ref[pl.ds(mult(r0 + r, 16), 16), :].astype(f32)
                p = wf * jnp.concatenate([col[r:r + 16]] * (D // 128), axis=1)
                acc = acc + (p[:8] + p[8:])
            return acc

        def down(acc, r0, n):
            return rows_dot(acc, wd_b, r0, h_s[pl.ds(mult(r0, 16), n), :])

        def head_tasks(h, st, cuts=(32, 32)):
            tasks = {}
            n = W // 4
            slot = h & (RING - 1)

            def qk(j):
                sl = slice(j * n, (j + 1) * n)
                s_s[:, sl] = jnp.dot(q_s[h].astype(bf16), k_b[slot, :, sl], preferred_element_type=f32)

            def softmax():
                sc = s_s[...] * (DH ** -0.5)
                e = jnp.exp(sc - jnp.max(sc, axis=-1, keepdims=True))
                s_s[...] = e / jnp.sum(e, axis=-1, keepdims=True)

            def pv(t0, t1):
                for t in range(t0, t1):
                    sl = slice(t * 128, (t + 1) * 128)
                    part = v_b[slot, :, sl].astype(f32) * jnp.concatenate([s_s[:, sl]] * (DH // M), axis=0)
                    st['o'] = part if t == 0 else st['o'] + part

            def proj():
                o = jnp.broadcast_to(jnp.sum(st['o'], axis=-1, keepdims=True), (DH, 128))
                st['a'] = rows_dot(a_s[...], wo_b, h * DH, o)
                a_s[...] = st['a']

            for j in range(4):
                tasks[1 + j] = [lambda j=j: qk(j)]
                tasks[6 + j] = [lambda j=j: pv(cuts[j], cuts[j + 1])]
            tasks[5] = [softmax]
            tasks[9].append(proj)
            return tasks

        def iteration(it, rep, tasks, gap, q0=None, q1=None):
            pieces = w_pieces(rep, it) if q0 is None else q0
            n0 = len(pieces)
            ns = STEPS if q1 is None else LAST_AT
            for s in range(STEPS):
                with scope(f"w{s}"):
                    kv(*piece(it, s)).wait()
                if q1 is None or s + LOOK < STEPS:
                    kv(*piece(it, s + LOOK)).start(priority=1)
                elif s + LOOK == STEPS:
                    for c in q1:
                        wcopy(*c).start(priority=1)
                for i, c in enumerate(pieces[s * n0 // ns:(s + 1) * n0 // ns]):
                    if i:
                        pl.delay(gap)
                    wcopy(*c).start(priority=0)
                if s == HALF:
                    w_wait(rep - 1, it - 1)
                if compute:
                    for t in tasks.get(s, []):
                        t()

        def loop(lo, hi, fn):
            assert len({(tuple(s[2] for s in active(i)), tuple(s[2] for s in active(i - 1))) for i in range(lo, hi)}) == 1
            if hi - lo == 1:
                fn(lo, lo)
            else:
                jax.lax.fori_loop(lo, hi, lambda i, c: fn(i, lo), None)

        kv(0, 0).start(priority=1)
        for c in small:
            c.start()
        kv(1, 0).start(priority=1)
        for s in range(LOOK):
            kv(*piece(0, s)).start(priority=1)
        first = w_pieces(0, 0)
        for c in first[:PRE0]:
            pl.delay(GAP0)
            wcopy(*c).start(priority=0)
        a_s[...] = jnp.zeros_like(a_s)
        y_s[...] = jnp.zeros_like(y_s)
        for c in small:
            c.wait()
        kv(0, 0).wait()
        kv(1, 0).wait()
        iteration(0, 0, {}, GAP_P, q0=first[PRE0:])
        loop(1, N_P, lambda it, rep: iteration(it, rep, {}, GAP_P))
        iteration(N_P, N_P, {}, GAP_P)
        for it in (N_P + 1, N_P + 2):
            iteration(it, it, {s: [lambda s=s: q_block((it - N_P - 1) * 8 + s - 1)] for s in range(1, 9)}, GAP)

        def head_it(first=None, mid=None):
            def fn(it, rep):
                tasks = head_tasks(it - J0, {}, (0, 10, 20, 30, 32))
                if first:
                    tasks[0] = [lambda: first(it)]
                if mid:
                    tasks[5].append(lambda: mid(it))
                iteration(it, rep, tasks, GAP)
            return fn

        def down_block(it):
            y_s[...] = down(y_s[...], (it - (N_P + 28)) * 128, 128)

        loop(J0, N_P + 10, head_it())
        loop(N_P + 10, N_P + 11, head_it())
        loop(N_P + 11, N_P + 20, head_it())
        loop(N_P + 20, N_P + 21, head_it())
        loop(N_P + 21, N_IT - 1, head_it(
            lambda it: pl.when(it < N_P + 27)(lambda: gu_block(it - (N_P + 21))),
            lambda it: pl.when(it >= N_P + 28)(lambda: down_block(it))))

        it = N_IT - 1
        st = {}
        tasks = head_tasks(H - 1, st, (0, 12, 22, 28, 32))
        tasks[5].append(lambda: down_block(it))
        xf = x_v[0].astype(f32)
        gate = jax.nn.sigmoid(jnp.sum(xf * gw_v[...].astype(f32).reshape(1, D), axis=-1, keepdims=True))
        rsel = jax.nn.sigmoid(jnp.sum(xf * wr_v[...].astype(f32).reshape(1, D), axis=-1, keepdims=True))
        groups, r = [], wd_main
        for g, n in enumerate((wd_last,) + tuple(TAIL)):
            groups.append((wd, wd_b, r, n, 0, D, e_sem.at[g]))
            r += n
        iteration(it, it, tasks, LAST_GAP,
                  q0=[(wd, wd_b, wd_main + r, 1, 0, D, e_sem.at[0]) for r in range(wd_last)], q1=groups[1:])
        y = y_s[...]
        for g, c in enumerate(groups):
            with scope(f"e{g}"):
                wcopy(*c).wait()
            if compute:
                y = down(y, 8 * c[2], 8 * c[3])
        a = jnp.sum(st['a'] if compute else y, axis=0, keepdims=True)
        y = jnp.sum(y, axis=0, keepdims=True)
        b = xf + (xf * 0.0 + y * rsel)
        out_ref[0] = (gate * a + (1.0 - gate) * b).astype(bf16)

    def fn(A_x, A_k_cache, A_v_cache, A_wq, A_wo, B_x, B_w_r, B_w_gate, B_w_up, B_w_down, gate_w):
        del B_x
        kT = jnp.swapaxes(A_k_cache, 2, 3)
        vT = jnp.swapaxes(A_v_cache, 2, 3)
        vmem = pltpu.VMEM
        dma = pltpu.SemaphoreType.DMA
        return pl.pallas_call(
            kernel,
            out_shape=jax.ShapeDtypeStruct((1, 1, D), bf16),
            in_specs=[pl.BlockSpec(memory_space=pl.ANY)] * 10,
            out_specs=pl.BlockSpec(memory_space=pltpu.VMEM),
            scratch_shapes=[
                vmem((1, 1, D), bf16), vmem((D,), bf16), vmem((D,), bf16),
                vmem((D, H * DH), bf16), vmem((RING, DH, W), bf16), vmem((RING, DH, W), bf16),
                vmem((H * DH, D), bf16), vmem((D, F), bf16), vmem((D, F), bf16), vmem((F, D), bf16),
                vmem((H, M, DH), f32), vmem((M, W), f32), vmem((M, D), f32), vmem((M, D), f32),
                vmem((F, 128), f32),
                dma((2, 8)), dma((2, 2)), dma((3,)), dma((len(TAIL) + 1,)),
            ],
            compiler_params=pltpu.CompilerParams(
                vmem_limit_bytes=100 * 1024 * 1024,
                disable_semaphore_checks=True,
                disable_bounds_checks=True,
            ),
            name="gated_mix_decode",
        )(A_x, kT, vT, A_wq, A_wo, B_w_r, B_w_gate, B_w_up, B_w_down, gate_w)

    return fn


_fn = make(GAP=30, GAP_P=40)


@jax.jit
def pallas_gated_mix__sliding_block_cached__moe_arch_mod__decode_kernel(
        A_x, A_k_cache, A_v_cache, A_wq, A_wo, B_x, B_w_r, B_w_gate, B_w_up, B_w_down, gate_w):
    return _fn(A_x, A_k_cache, A_v_cache, A_wq, A_wo, B_x, B_w_r, B_w_gate, B_w_up, B_w_down, gate_w)
```

```python
import jax
import jax.numpy as jnp
import jax.experimental.pallas as pl
import jax.experimental.pallas.tpu as pltpu

H, DH, SK, D, F = 32, 192, 32768, 640, 1536
W = min(4096, max(256, SK // 4))
BASE = SK - W
DT = D // 128

STEPS = 8
RING = 4
PIECE = 32
LEAD = 3
TAIL = (8, 8, 8, 8, 8, 4, 2, 2)
GAP_IDLE = 45
GAP_BUSY = 20
IT_GU, IT_O, IT_D = 24, 34, 58
IT_PROJ = 2 * H - H // 2

f32 = jnp.float32
bf16 = jnp.bfloat16


def _mult(i, n):
    return i if isinstance(i, int) else pl.multiple_of(i, n)


def _column(row):
    return jnp.broadcast_to(row, (128, 128)).T


def _tiles(ref, first, n):
    out = []
    for i in range(0, n, 2):
        w = ref[pl.ds(_mult(8 * (first + i), 16), 16), :].astype(f32)
        out += [w[:8], w[8:]]
    return out


def _kernel(x_hbm, kT, vT, wq, wo, wr_hbm, wg, wu, wd, gw_hbm, out_ref,
            x_v, wr_v, gw_v, wq_b, k_b, v_b, wo_b, wg_b, wu_b, wd_b,
            x_c, q_c, h_c, p_s, a_s, y_s, kv_sem, w_sem, d_sem, s_sem, e_sem):
    def kv(which, h, s):
        rows, c = pl.ds(8 * (s // 4), 8), (W // 4) * (s % 4)
        src = (kT, vT)[which].at[h, :, rows, pl.ds(BASE + c, W // 4)]
        dst = k_b.at[h] if which == 0 else v_b.at[h & (RING - 1)]
        return pltpu.make_async_copy(src, dst.at[:, rows, pl.ds(c, W // 4)], kv_sem.at[s])

    def piece(src, dst, p, sem):
        rows = pl.ds(_mult(p * PIECE, PIECE), PIECE)
        return pltpu.make_async_copy(src.at[rows], dst.at[rows], sem)

    def q_pieces(t):
        return [piece(wq, wq_b, (5 * (t >> 6) + j) * 64 + (t & 63), w_sem.at[0]) for j in range(5)]

    def gu_pieces(t):
        return [piece(src, dst, 80 * j + t, w_sem.at[k])
                for j in range(3) for src, dst, k in ((wg, wg_b, 1), (wu, wu_b, 2))]

    def o_pieces(t):
        return [piece(wo, wo_b, (5 * (t >> 6) + j) * 64 + (t & 63), w_sem.at[3 + (t >> 6)]) for j in range(5)]

    def d_pieces(t, group):
        return [piece(wd.at[j], wd_b.at[j], t, d_sem.at[group]) for j in range(4)]

    def d_rows(first, n):
        return (slice(None), pl.ds(_mult(8 * first, 8), 8 * n))

    def landed(buf, sem):
        pltpu.make_async_copy(buf, buf, sem).wait()

    def iteration(it, which, nxt, weights, tasks, gap):
        for s in range(STEPS):
            kv(which, it & (H - 1), s).wait()
            for c in nxt(s):
                c.start(priority=1)
            todo = list(tasks.get(s, []))
            for i, c in enumerate(weights(s)):
                if i and todo:
                    pl.delay(1)
                    todo.pop(0)()
                    pl.delay(1)
                elif i:
                    pl.delay(gap)
                c.start(priority=0)
            for task in todo:
                task()

    def loop(lo, hi, fn):
        jax.lax.fori_loop(lo, hi, lambda i, c: fn(i), None)

    def x_dot(w_ref, width, b, acc, n):
        def part(k):
            for rt in range(k * (D // 8) // n, (k + 1) * (D // 8) // n):
                xc = x_c[8 * rt:8 * rt + 8, :]
                p = [w * xc for w in _tiles(w_ref, rt * width + 2 * b, 2)]
                acc[:] = [u + v for u, v in zip(acc, p)] if rt else p
        return [lambda k=k: part(k) for k in range(n)]

    def q_block(b):
        q = []

        def store():
            for i in range(2):
                q_c[pl.ds(_mult((2 * b + i) * 128, 128), 128), :] = _column(jnp.sum(q[i], axis=0, keepdims=True))
        return x_dot(wq_b, H * DH // 128, b, q, 5) + [store]

    def gate_block(b):
        g = []
        x_dot(wg_b, F // 128, b, g, 1)[0]()
        for i in range(2):
            h_c[pl.ds(_mult((2 * b + i) * 128, 128), 8), :] = jnp.broadcast_to(
                jax.nn.silu(jnp.sum(g[i], axis=0, keepdims=True)), (8, 128))

    def up_block(b):
        u = []
        x_dot(wu_b, F // 128, b, u, 1)[0]()
        for i in range(2):
            r = _mult((2 * b + i) * 128, 128)
            h_c[pl.ds(r, 128), :] = _column(h_c[pl.ds(r, 8), :][:1] * jnp.sum(u[i], axis=0, keepdims=True))

    def split(a):
        return [a[:, c:c + 128] for c in range(0, D, 128)]

    def proj(h, o=None):
        o = q_c[pl.ds(_mult(h * DH, DH), DH), :] if o is None else o
        acc = split(a_s[...])
        for t, w in enumerate(_tiles(wo_b, h * (DH // 8 * DT), DH // 8 * DT)):
            acc[t % DT] = acc[t % DT] + w * o[8 * (t // DT):8 * (t // DT) + 8]
        a_s[...] = jnp.concatenate(acc, axis=1)

    def down(acc, rt, first, n):
        for j in range(4):
            for t, w in enumerate(_tiles(wd_b.at[j], DT * rt + first, n), first):
                rows = pl.ds(_mult(j * (F // 4) + 8 * (rt + t // DT), 8), 8)
                acc[t % DT] = acc[t % DT] + w * h_c[rows, :]
        return acc

    def attention(h, st):
        head = pl.ds(_mult(h * DH, DH), DH)

        def qk(j):
            q = q_c[head, :]
            for c in range(256 * j, 256 * (j + 1), 128):
                k = k_b[h, :, :, c:c + 128].reshape(DH, 128).astype(f32)
                p_s[:, c:c + 128] = jnp.broadcast_to(jnp.sum(k * q, axis=0, keepdims=True), (8, 128))

        def softmax():
            s = p_s[...] * (DH ** -0.5)
            e = jnp.exp(s - jnp.max(s, axis=-1, keepdims=True))
            p_s[...] = e / jnp.sum(e, axis=-1, keepdims=True)

        def pv(j):
            for c in range(256 * j, 256 * (j + 1), 128):
                v = v_b[h & (RING - 1), :, :, c:c + 128].reshape(DH, 128).astype(f32)
                part = v * jnp.concatenate([p_s[:, c:c + 128]] * (DH // 8), axis=0)
                st['o'] = st['o'] + part if c else part

        def finish():
            st['o'] = jnp.broadcast_to(jnp.sum(st['o'], axis=-1, keepdims=True), (DH, 128))
            q_c[head, :] = st['o']

        tasks = {s: [lambda j=4 * s + i: qk(j) for i in range(4)] for s in range(4)}
        tasks.update({4 + s: [lambda j=4 * s + i: pv(j) for i in range(4)] for s in range(4)})
        tasks[3].append(softmax)
        tasks[7].append(finish)
        return tasks

    def k_iteration(it, weights, tasks, gap, last=False):
        iteration(it, 0, lambda s: [kv(int(last), (it + 1) & (H - 1), s)], weights, tasks, gap)

    small = [pltpu.make_async_copy(x_hbm, x_v, s_sem.at[0]),
             pltpu.make_async_copy(gw_hbm, gw_v, s_sem.at[1]),
             pltpu.make_async_copy(wr_hbm, wr_v, s_sem.at[2])]
    kv(0, 0, 0).start(priority=1)
    for c in small:
        c.start()
    for s in range(1, STEPS):
        kv(0, 0, s).start(priority=1)
    for t in range(LEAD):
        for c in q_pieces(t):
            c.start(priority=0)
            pl.delay(GAP_BUSY)
    loop(0, IT_GU - 1, lambda it: k_iteration(it, lambda s: q_pieces(STEPS * it + s + LEAD), {}, GAP_IDLE))

    for c in small:
        c.wait()
    a_s[...] = jnp.zeros_like(a_s)
    y_s[...] = jnp.zeros_like(y_s)
    for c in range(0, D, 128):
        x_c[c:c + 128, :] = _column(x_v[0, :, c:c + 128].astype(f32))
    k_iteration(IT_GU - 1, lambda s: (q_pieces(STEPS * (IT_GU - 1) + s + LEAD) if s + LEAD < STEPS
                                      else d_pieces(s + LEAD - STEPS, 0)), {}, GAP_BUSY)

    def gu_feed(it):
        return lambda s: gu_pieces(STEPS * (it - IT_GU) + s)

    k_iteration(IT_GU, gu_feed(IT_GU), {}, GAP_IDLE * 4 // 5)
    landed(wq_b, w_sem.at[0])
    landed(wd_b.at[d_rows(0, 4 * LEAD)], d_sem.at[0])
    loop(IT_GU + 1, H - 1, lambda it: k_iteration(
        it, gu_feed(it), {2 * j: q_block(4 * (it - IT_GU - 1) + j) for j in range(4)}, GAP_BUSY))
    k_iteration(H - 1, gu_feed(H - 1), {}, GAP_IDLE * 4 // 5, last=True)

    def v_iteration(it, weights, extra, nxt=None):
        st = {}
        tasks = attention(it - H, st)
        for s, task in extra(st):
            tasks[s].append(task)
        iteration(it, 1, nxt or (lambda s: [kv(1, it + 1 - H, s)]), weights, tasks, GAP_BUSY)

    def o_landed(it):
        g, n = (it - IT_O - STEPS) >> 3, wo_b.shape[0] // 3
        landed(wo_b.at[pl.ds(_mult(g * n, 16), n)], w_sem.at[3 + g])

    def o_extra(it):
        b, h = it - IT_O - 1, 2 * (it - IT_PROJ)

        def first():
            @pl.when(it == IT_O)
            def _():
                landed(wg_b, w_sem.at[1])
                landed(wu_b, w_sem.at[2])
            pl.when((it > IT_O) & ((it - IT_O) & 7 == 0))(lambda: o_landed(it))
            pl.when((b >= 0) & (b < 6))(lambda: gate_block(b))
            pl.when((b >= 6) & (b < 12))(lambda: up_block(b - 6))
            pl.when(h >= 0)(lambda: proj(h))
        return lambda st: [(5, first), (7, lambda: pl.when(h >= 0)(lambda: proj(h + 1)))]

    def d_feed(it):
        return lambda s: d_pieces(STEPS * (it - IT_D) + s + LEAD, it - IT_D + 1)

    def down_block(it):
        i = it - IT_D - 1
        landed(wd_b.at[d_rows(4 * LEAD + 32 * i, 32)], d_sem.at[i + 1])
        y_s[...] = jnp.concatenate(down(split(y_s[...]), 6 * i, 0, 6 * DT), axis=1)

    def d_extra(it):
        h = 2 * (it - IT_PROJ)

        def first():
            pl.when(it == IT_D)(lambda: o_landed(it))
            pl.when(it > IT_D)(lambda: down_block(it))
        return lambda st: [(4, first), (5, lambda: proj(h)), (7, lambda: proj(h + 1))]

    loop(H, IT_O, lambda it: v_iteration(it, gu_feed(it), lambda st: []))
    loop(IT_O, IT_D, lambda it: v_iteration(it, lambda s: o_pieces(STEPS * (it - IT_O) + s), o_extra(it)))
    loop(IT_D, 2 * H - 1, lambda it: v_iteration(it, d_feed(it), d_extra(it)))

    xf = x_v[0].astype(f32)
    gate = jax.nn.sigmoid(jnp.sum(xf * gw_v[...].astype(f32).reshape(1, D), axis=-1, keepdims=True))
    rsel = jax.nn.sigmoid(jnp.sum(xf * wr_v[...].astype(f32).reshape(1, D), axis=-1, keepdims=True))

    it = 2 * H - 1
    fed = 4 * STEPS * (2 * H - IT_D)
    tail, t = [], fed
    for g, n in enumerate(TAIL):
        tail.append((t, n, pltpu.make_async_copy(wd.at[d_rows(t, n)], wd_b.at[d_rows(t, n)], e_sem.at[g])))
        t += n
    assert 8 * t == wd.shape[1]
    v_iteration(it, lambda s: d_feed(it)(s) if s + LEAD < STEPS else [],
                lambda st: [(1, lambda: proj(H - 2)), (2, lambda: down_block(it)),
                            (7, lambda: proj(H - 1, st['o']))],
                lambda s: [] if s else [c for _, _, c in tail])

    n = 4 * (STEPS - LEAD)
    landed(wd_b.at[d_rows(fed - n, n)], d_sem.at[it - IT_D + 1])
    done = 6 * DT * (it - IT_D)
    y = down(split(y_s[...]), 0, done, fed - done)
    a = jnp.sum(a_s[...], axis=0, keepdims=True)
    for t, n, c in tail:
        c.wait()
        y = down(y, 0, t, n)
    y = jnp.sum(jnp.concatenate(y, axis=1), axis=0, keepdims=True)
    b = xf + (xf * 0.0 + y * rsel)
    out_ref[0] = (gate * a + (1.0 - gate) * b).astype(bf16)


def _tile_list(w):
    r, c = w.shape
    return w.reshape(r // 8, 8, c // 128, 128).transpose(0, 2, 1, 3).reshape(-1, 128)


@jax.jit
def pallas_gated_mix__sliding_block_cached__moe_arch_mod__decode_kernel(
        A_x, A_k_cache, A_v_cache, A_wq, A_wo, B_x, B_w_r, B_w_gate, B_w_up, B_w_down, gate_w):
    del B_x
    kT = jnp.swapaxes(A_k_cache, 2, 3).reshape(H, DH // 16, 16, SK)
    vT = jnp.swapaxes(A_v_cache, 2, 3).reshape(H, DH // 16, 16, SK)
    wq, wo, wg, wu = (_tile_list(w) for w in (A_wq, A_wo, B_w_gate, B_w_up))
    wd = _tile_list(B_w_down).reshape(4, -1, 128)
    vmem = pltpu.VMEM
    dma = pltpu.SemaphoreType.DMA
    return pl.pallas_call(
        _kernel,
        out_shape=jax.ShapeDtypeStruct((1, 1, D), bf16),
        in_specs=[pl.BlockSpec(memory_space=pl.ANY)] * 10,
        out_specs=pl.BlockSpec(memory_space=pltpu.VMEM),
        scratch_shapes=[
            vmem((1, 1, D), bf16), vmem((D,), bf16), vmem((D,), bf16),
            vmem(wq.shape, bf16), vmem((H, DH // 16, 16, W), bf16), vmem((RING, DH // 16, 16, W), bf16),
            vmem(wo.shape, bf16), vmem(wg.shape, bf16), vmem(wu.shape, bf16), vmem(wd.shape, bf16),
            vmem((D, 128), f32), vmem((H * DH, 128), f32), vmem((F, 128), f32),
            vmem((8, W), f32), vmem((8, D), f32), vmem((8, D), f32),
            dma((STEPS,)), dma((6,)), dma((2 * H - IT_D + 1,)), dma((3,)), dma((len(TAIL),)),
        ],
        compiler_params=pltpu.CompilerParams(
            vmem_limit_bytes=100 * 1024 * 1024,
            disable_semaphore_checks=True,
            disable_bounds_checks=True,
        ),
        name="gated_mix_decode",
    )(A_x, kT, vT, wq, wo, B_w_r, wg, wu, wd, gate_w)
```

```python
import jax
import jax.numpy as jnp
import jax.experimental.pallas as pl
import jax.experimental.pallas.tpu as pltpu

H, DH, SK, D, F = 32, 192, 32768, 640, 1536
W = min(4096, max(256, SK // 4))
BASE = SK - W
DT = D // 128

STEPS = 8
RING = 4
PIECE = 32
FEED = 40
LEAD = 16
LAST = (6, 2)
TAIL = (16, 16, 8, 8, 8, 8, 4, 4)
GAP_IDLE = 45
GAP_BUSY = 25
IT_GU, IT_O, IT_D = 24, 36, 60
IT_PROJ = 2 * H - H // 2

f32 = jnp.float32
bf16 = jnp.bfloat16


def _mult(i, n):
    return i if isinstance(i, int) else pl.multiple_of(i, n)


def _column(row):
    return jnp.broadcast_to(row, (128, 128)).T


def _tiles(ref, first, n):
    out = []
    for i in range(0, n, 2):
        w = ref[pl.ds(_mult(8 * (first + i), 16), 16), :].astype(f32)
        out += [w[:8], w[8:]]
    return out


def _kernel(x_hbm, kT, vT, wq, wo, wr_hbm, wg, wu, wd, gw_hbm, out_ref,
            x_v, wr_v, gw_v, wq_b, k_b, v_b, wo_b, wg_b, wu_b, wd_b,
            x_c, q_c, h_c, p_s, a_s, y_s, kv_sem, w_sem, s_sem, e_sem):
    def kv(which, h, s):
        rows, c = pl.ds(8 * (s // 4), 8), (W // 4) * (3 - s if s < 4 else s - 4)
        src = (kT, vT)[which].at[h, :, rows, pl.ds(BASE + c, W // 4)]
        dst = k_b.at[h] if which == 0 else v_b.at[h & (RING - 1)]
        return pltpu.make_async_copy(src, dst.at[:, rows, pl.ds(c, W // 4)], kv_sem.at[s])

    def pieces(parts, first, n, sem):
        out = []
        for i in range(0, n, 2):
            for src, dst in parts:
                for p in (first + i, first + i + 1):
                    rows = pl.ds(_mult(p * PIECE, PIECE), PIECE)
                    out.append(pltpu.make_async_copy(src.at[rows], dst.at[rows], sem))
        return out

    def parts(src, dst):
        return [(src.at[j], dst.at[j]) for j in range(src.shape[0])]

    def tile_rows(first, n):
        return (slice(None), pl.ds(_mult(8 * first, 8), 8 * n))

    def landed(buf, sem):
        pltpu.make_async_copy(buf, buf, sem).wait()

    def iteration(it, which, nxt, feed, tasks, gap):
        for s in range(STEPS):
            kv(which, it & (H - 1), s).wait()
            for c in nxt(s):
                c.start(priority=1)
            todo = list(tasks.get(s, []))
            for i, c in enumerate(feed[s * FEED // STEPS:(s + 1) * FEED // STEPS]):
                if i and todo:
                    pl.delay(1)
                    todo.pop(0)()
                    pl.delay(1)
                elif i:
                    pl.delay(gap)
                c.start(priority=0)
            for task in todo:
                task()

    def loop(lo, hi, fn):
        jax.lax.fori_loop(lo, hi, lambda i, c: fn(i), None)

    def x_dot(w_refs, width, b, acc, n):
        def part(k):
            for rt in range(k * (D // 8) // n, (k + 1) * (D // 8) // n):
                xc = x_c[8 * rt:8 * rt + 8, :]
                j, r = divmod(rt, D // 8 // len(w_refs))
                p = [w * xc for w in _tiles(w_refs[j], r * width + 2 * b, 2)]
                acc[:] = [u + v for u, v in zip(acc, p)] if rt else p
        return [lambda k=k: part(k) for k in range(n)]

    def q_block(b):
        q = []

        def store():
            for i in range(2):
                q_c[pl.ds(_mult((2 * b + i) * 128, 128), 128), :] = _column(jnp.sum(q[i], axis=0, keepdims=True))
        return x_dot([wq_b.at[0], wq_b.at[1]], H * DH // 128, b, q, 4) + [store]

    def gate_block(b):
        g = []
        x_dot([wg_b], F // 128, b, g, 1)[0]()
        for i in range(2):
            h_c[pl.ds(_mult((2 * b + i) * 128, 128), 8), :] = jnp.broadcast_to(
                jax.nn.silu(jnp.sum(g[i], axis=0, keepdims=True)), (8, 128))

    def up_block(b):
        u = []
        x_dot([wu_b], F // 128, b, u, 1)[0]()
        for i in range(2):
            r = _mult((2 * b + i) * 128, 128)
            h_c[pl.ds(r, 128), :] = _column(h_c[pl.ds(r, 8), :][:1] * jnp.sum(u[i], axis=0, keepdims=True))

    def split(a):
        return [a[:, c:c + 128] for c in range(0, D, 128)]

    def proj(half, h, o):
        acc = split(a_s[...])
        for t, w in enumerate(_tiles(wo_b.at[half], h * (DH // 8 * DT), DH // 8 * DT)):
            acc[t % DT] = acc[t % DT] + w * o[8 * (t // DT):8 * (t // DT) + 8]
        a_s[...] = jnp.concatenate(acc, axis=1)

    def down(acc, rt, first, n):
        for j in range(4):
            for t, w in enumerate(_tiles(wd_b.at[j], DT * rt + first, n), first):
                rows = pl.ds(_mult(j * (F // 4) + 8 * (rt + t // DT), 8), 8)
                acc[t % DT] = acc[t % DT] + w * h_c[rows, :]
        return acc

    def attention(h, st):
        head = pl.ds(_mult(h * DH, DH), DH)

        def qk(j):
            q = q_c[head, :]
            for c in range(256 * j, 256 * (j + 1), 128):
                k = k_b[h, :, :, c:c + 128].reshape(DH, 128).astype(f32)
                p_s[:, c:c + 128] = jnp.broadcast_to(jnp.sum(k * q, axis=0, keepdims=True), (8, 128))

        def softmax():
            s = p_s[...] * (DH ** -0.5)
            e = jnp.exp(s - jnp.max(s, axis=-1, keepdims=True))
            p_s[...] = e / jnp.sum(e, axis=-1, keepdims=True)

        def pv(j):
            for c in range(256 * j, 256 * (j + 1), 128):
                v = v_b[h & (RING - 1), :, :, c:c + 128].reshape(DH, 128).astype(f32)
                part = v * jnp.concatenate([p_s[:, c:c + 128]] * (DH // 8), axis=0)
                st['o'] = st['o'] + part if c else part

        def finish():
            st['o'] = jnp.broadcast_to(jnp.sum(st['o'], axis=-1, keepdims=True), (DH, 128))

        tasks = {s: [lambda j=4 * s + i: qk(j) for i in range(4)] for s in range(4)}
        tasks.update({4 + s: [lambda j=4 * s + i: pv(j) for i in range(4)] for s in range(4)})
        tasks[3].append(softmax)
        tasks[7].append(finish)
        return tasks

    def k_iteration(it, feed, tasks=None, last=False):
        iteration(it, 0, lambda s: [kv(int(last), (it + 1) & (H - 1), s)], feed, tasks or {},
                  GAP_IDLE if tasks is None else GAP_BUSY)

    def q_feed(first, n):
        return pieces(parts(wq, wq_b), first, n, w_sem.at[0])

    def gu_feed(it):
        return pieces([(wg, wg_b), (wu, wu_b)], FEED // 2 * (it - IT_GU), FEED // 2, w_sem.at[1])

    small = [pltpu.make_async_copy(x_hbm, x_v, s_sem.at[0]),
             pltpu.make_async_copy(gw_hbm, gw_v, s_sem.at[1]),
             pltpu.make_async_copy(wr_hbm, wr_v, s_sem.at[2])]
    kv(0, 0, 0).start(priority=1)
    for c in small:
        c.start()
    for s in range(1, STEPS):
        kv(0, 0, s).start(priority=1)
    for c in q_feed(0, LEAD // 2):
        c.start(priority=0)
        pl.delay(35)
    loop(0, IT_GU - 1, lambda it: k_iteration(it, q_feed((LEAD + FEED * it) // 2, FEED // 2)))

    for c in small:
        c.wait()
    a_s[...] = jnp.zeros_like(a_s)
    for c in range(0, D, 128):
        x_c[c:c + 128, :] = _column(x_v[0, :, c:c + 128].astype(f32))
    d_lead = FEED // 4 * (2 * H - 1 - IT_D)
    k_iteration(IT_GU - 1, q_feed((LEAD + FEED * (IT_GU - 1)) // 2, (FEED - LEAD) // 2)
                + pieces(parts(wd, wd_b), d_lead, LEAD // 4, w_sem.at[2]), {})
    k_iteration(IT_GU, gu_feed(IT_GU))
    landed(wq_b, w_sem.at[0])
    landed(wd_b.at[tile_rows(4 * d_lead, LEAD)], w_sem.at[2])
    loop(IT_GU + 1, H - 1, lambda it: k_iteration(
        it, gu_feed(it), {2 * j: q_block(4 * (it - IT_GU - 1) + j) for j in range(4)}))
    k_iteration(H - 1, gu_feed(H - 1), last=True)

    def v_iteration(it, feed, extra, project, nxt=None):
        st = {}
        tasks = attention(it - H, st)
        for s, task in extra:
            tasks[s].append(task)
        if project:
            h = it - IT_PROJ
            tasks[project].append(lambda: proj(0, h, q_c[pl.ds(_mult(h * DH, DH), DH), :]))
            tasks[7].append(lambda: proj(1, h, st['o']))
        else:
            def keep():
                q_c[pl.ds(_mult((it - H) * DH, DH), DH), :] = st['o']
            tasks[7].append(keep)
        iteration(it, 1, nxt or (lambda s: [kv(1, it + 1 - H, s)]), feed, tasks, GAP_BUSY)

    def o_feed(it):
        return pieces(parts(wo, wo_b), FEED // 2 * (it - IT_O), FEED // 2, w_sem.at[3 + (it & 1)])

    def o_landed(it):
        landed(wo_b.at[tile_rows(2 * FEED * (it - IT_O), 2 * FEED)], w_sem.at[3 + (it & 1)])

    def ffn_block(it):
        @pl.when(it == IT_O)
        def _():
            landed(wg_b, w_sem.at[1])
            landed(wu_b, w_sem.at[1])
        pl.when(it > IT_O)(lambda: o_landed(it - 1))
        pl.when(it < IT_O + 6)(lambda: gate_block(it - IT_O))
        pl.when(it >= IT_O + 6)(lambda: up_block(it - IT_O - 6))

    def d_feed(it):
        return pieces(parts(wd, wd_b), FEED // 4 * (it - IT_D), FEED // 4, w_sem.at[3 + (it & 1)])

    def down_block(it):
        landed(wd_b.at[tile_rows(FEED * (it - IT_D), FEED)], w_sem.at[3 + (it & 1)])
        y_s[...] = jnp.concatenate(down(split(y_s[...]), FEED // DT * (it - IT_D), 0, FEED), axis=1)

    def d_block(it):
        @pl.when(it == IT_D)
        def _():
            o_landed(it - 1)
            y_s[...] = jnp.concatenate(down(split(jnp.zeros((8, D), f32)), 0, 4 * d_lead, LEAD), axis=1)
        pl.when(it > IT_D)(lambda: down_block(it - 1))

    loop(H, IT_O, lambda it: v_iteration(it, gu_feed(it), [], None))
    loop(IT_O, IT_PROJ, lambda it: v_iteration(it, o_feed(it), [(5, lambda: ffn_block(it))], None))
    loop(IT_PROJ, IT_D, lambda it: v_iteration(it, o_feed(it), [(4, lambda: o_landed(it - 1))], 5))
    loop(IT_D, 2 * H - 1, lambda it: v_iteration(it, d_feed(it), [(4, lambda: d_block(it))], 5))

    xf = x_v[0].astype(f32)
    gate = jax.nn.sigmoid(jnp.sum(xf * gw_v[...].astype(f32).reshape(1, D), axis=-1, keepdims=True))
    rsel = jax.nn.sigmoid(jnp.sum(xf * wr_v[...].astype(f32).reshape(1, D), axis=-1, keepdims=True))

    it = 2 * H - 1
    feed, rest, t = [], [], 4 * d_lead + LEAD
    for g, n in enumerate(LAST + TAIL):
        if g < len(LAST):
            feed += pieces(parts(wd, wd_b), t // 4, n, e_sem.at[g])
            n *= 4
        rest.append((t, n, pltpu.make_async_copy(wd.at[tile_rows(t, n)], wd_b.at[tile_rows(t, n)], e_sem.at[g])))
        t += n
    assert 8 * t == wd.shape[1] and len(feed) <= FEED
    v_iteration(it, feed, [(2, lambda: down_block(it - 1))], 1,
                lambda s: [] if s else [c for _, _, c in rest[len(LAST):]])

    a = jnp.sum(a_s[...], axis=0, keepdims=True)
    y = split(y_s[...])
    for t, n, c in rest:
        c.wait()
        y = down(y, 0, t, n)
    y = jnp.sum(jnp.concatenate(y, axis=1), axis=0, keepdims=True)
    b = xf + (xf * 0.0 + y * rsel)
    out_ref[0] = (gate * a + (1.0 - gate) * b).astype(bf16)


def _tile_list(w):
    r, c = w.shape
    return w.reshape(r // 8, 8, c // 128, 128).transpose(0, 2, 1, 3).reshape(-1, 128)


@jax.jit
def pallas_gated_mix__sliding_block_cached__moe_arch_mod__decode_kernel(
        A_x, A_k_cache, A_v_cache, A_wq, A_wo, B_x, B_w_r, B_w_gate, B_w_up, B_w_down, gate_w):
    del B_x
    kT = jnp.swapaxes(A_k_cache, 2, 3).reshape(H, DH // 16, 16, SK)
    vT = jnp.swapaxes(A_v_cache, 2, 3).reshape(H, DH // 16, 16, SK)
    wg, wu = _tile_list(B_w_gate), _tile_list(B_w_up)
    wq, wo = _tile_list(A_wq).reshape(2, -1, 128), _tile_list(A_wo).reshape(2, -1, 128)
    wd = _tile_list(B_w_down).reshape(4, -1, 128)
    vmem = pltpu.VMEM
    dma = pltpu.SemaphoreType.DMA
    return pl.pallas_call(
        _kernel,
        out_shape=jax.ShapeDtypeStruct((1, 1, D), bf16),
        in_specs=[pl.BlockSpec(memory_space=pl.ANY)] * 10,
        out_specs=pl.BlockSpec(memory_space=pltpu.VMEM),
        scratch_shapes=[
            vmem((1, 1, D), bf16), vmem((D,), bf16), vmem((D,), bf16),
            vmem(wq.shape, bf16), vmem((H, DH // 16, 16, W), bf16), vmem((RING, DH // 16, 16, W), bf16),
            vmem(wo.shape, bf16), vmem(wg.shape, bf16), vmem(wu.shape, bf16), vmem(wd.shape, bf16),
            vmem((D, 128), f32), vmem((H * DH, 128), f32), vmem((F, 128), f32),
            vmem((8, W), f32), vmem((8, D), f32), vmem((8, D), f32),
            dma((STEPS,)), dma((5,)), dma((3,)), dma((len(LAST + TAIL),)),
        ],
        compiler_params=pltpu.CompilerParams(
            vmem_limit_bytes=100 * 1024 * 1024,
            disable_semaphore_checks=True,
            disable_bounds_checks=True,
        ),
        name="gated_mix_decode",
    )(A_x, kT, vT, wq, wo, B_w_r, wg, wu, wd, gate_w)
```

```python
import jax
import jax.numpy as jnp
import jax.experimental.pallas as pl
import jax.experimental.pallas.tpu as pltpu

H, DH, SK, D, F = 32, 192, 32768, 640, 1536
W = min(4096, max(256, SK // 4))
BASE = SK - W
DT = D // 128

STEPS = 8
RING = 4
PIECE = 32
FEED = 40
LEAD = 32
LAST = 24
TAIL = (24, 16, 12, 8, 4)
GAP_IDLE = 45
GAP_BUSY = 25
IT_GU, IT_O, IT_D = 24, 36, 60
IT_PROJ = 2 * H - H // 2

f32 = jnp.float32
bf16 = jnp.bfloat16


def _mult(i, n):
    return i if isinstance(i, int) else pl.multiple_of(i, n)


def _column(row):
    return jnp.broadcast_to(row, (128, 128)).T


def _tiles(ref, first, n):
    out = []
    for i in range(0, n, 2):
        w = ref[pl.ds(_mult(8 * (first + i), 16), 16), :].astype(f32)
        out += [w[:8], w[8:]]
    return out


def _kernel(x_hbm, kT, vT, wq, wo, wr_hbm, wg, wu, wd, gw_hbm, out_ref,
            x_v, wr_v, gw_v, wq_b, k_b, v_b, wo_b, wg_b, wu_b, wd_b,
            x_c, q_c, h_c, p_s, a_s, y_s, kv_sem, w_sem, s_sem, e_sem):
    def kv(which, h, s):
        rows, c = pl.ds(8 * (s // 4), 8), (W // 4) * (3 - s if s < 4 else s - 4)
        src = (kT, vT)[which].at[h, :, rows, pl.ds(BASE + c, W // 4)]
        dst = k_b.at[h] if which == 0 else v_b.at[h & (RING - 1)]
        return pltpu.make_async_copy(src, dst.at[:, rows, pl.ds(c, W // 4)], kv_sem.at[s])

    def pieces(parts, first, n, sem):
        out = []
        for i in range(0, n, 2):
            for src, dst in parts:
                for p in (first + i, first + i + 1):
                    rows = pl.ds(_mult(p * PIECE, PIECE), PIECE)
                    out.append(pltpu.make_async_copy(src.at[rows], dst.at[rows], sem))
        return out

    def parts(src, dst):
        return [(src.at[j], dst.at[j]) for j in range(src.shape[0])]

    def tile_rows(first, n):
        return (slice(None), pl.ds(_mult(8 * first, 8), 8 * n))

    def landed(buf, sem):
        pltpu.make_async_copy(buf, buf, sem).wait()

    def iteration(it, which, nxt, feed, tasks, gap):
        for s in range(STEPS):
            kv(which, it & (H - 1), s).wait()
            for c in nxt(s):
                c.start(priority=1)
            todo = list(tasks.get(s, []))
            for i, c in enumerate(feed[s * FEED // STEPS:(s + 1) * FEED // STEPS]):
                if i and todo:
                    pl.delay(1)
                    todo.pop(0)()
                    pl.delay(1)
                elif i:
                    pl.delay(gap)
                c.start(priority=0)
            for task in todo:
                task()

    def loop(lo, hi, fn):
        jax.lax.fori_loop(lo, hi, lambda i, c: fn(i), None)

    def x_dot(w_refs, width, b, acc, n):
        def part(k):
            for rt in range(k * (D // 8) // n, (k + 1) * (D // 8) // n):
                xc = x_c[8 * rt:8 * rt + 8, :]
                j, r = divmod(rt, D // 8 // len(w_refs))
                p = [w * xc for w in _tiles(w_refs[j], r * width + 2 * b, 2)]
                acc[:] = [u + v for u, v in zip(acc, p)] if rt else p
        return [lambda k=k: part(k) for k in range(n)]

    def q_block(b):
        q = []

        def store():
            for i in range(2):
                q_c[pl.ds(_mult((2 * b + i) * 128, 128), 128), :] = _column(jnp.sum(q[i], axis=0, keepdims=True))
        return x_dot([wq_b.at[0], wq_b.at[1]], H * DH // 128, b, q, 4) + [store]

    def gate_block(b):
        g = []
        x_dot([wg_b], F // 128, b, g, 1)[0]()
        for i in range(2):
            h_c[pl.ds(_mult((2 * b + i) * 128, 128), 8), :] = jnp.broadcast_to(
                jax.nn.silu(jnp.sum(g[i], axis=0, keepdims=True)), (8, 128))

    def up_block(b):
        u = []
        x_dot([wu_b], F // 128, b, u, 1)[0]()
        for i in range(2):
            r = _mult((2 * b + i) * 128, 128)
            h_c[pl.ds(r, 128), :] = _column(h_c[pl.ds(r, 8), :][:1] * jnp.sum(u[i], axis=0, keepdims=True))

    def split(a):
        return [a[:, c:c + 128] for c in range(0, D, 128)]

    def proj(half, h, o):
        acc = split(a_s[...])
        for t, w in enumerate(_tiles(wo_b.at[half], h * (DH // 8 * DT), DH // 8 * DT)):
            acc[t % DT] = acc[t % DT] + w * o[8 * (t // DT):8 * (t // DT) + 8]
        a_s[...] = jnp.concatenate(acc, axis=1)

    def down(acc, rt, first, n, quarters=range(4)):
        for j in quarters:
            for t, w in enumerate(_tiles(wd_b.at[j], DT * rt + first, n), first):
                rows = pl.ds(_mult(j * (F // 4) + 8 * (rt + t // DT), 8), 8)
                acc[t % DT] = acc[t % DT] + w * h_c[rows, :]
        return acc

    def attention(h, st):
        head = pl.ds(_mult(h * DH, DH), DH)

        def qk(j):
            q = q_c[head, :]
            for c in range(256 * j, 256 * (j + 1), 128):
                k = k_b[h, :, :, c:c + 128].reshape(DH, 128).astype(f32)
                p_s[:, c:c + 128] = jnp.broadcast_to(jnp.sum(k * q, axis=0, keepdims=True), (8, 128))

        def softmax():
            s = p_s[...] * (DH ** -0.5)
            e = jnp.exp(s - jnp.max(s, axis=-1, keepdims=True))
            p_s[...] = e / jnp.sum(e, axis=-1, keepdims=True)

        def pv(j):
            for c in range(256 * j, 256 * (j + 1), 128):
                v = v_b[h & (RING - 1), :, :, c:c + 128].reshape(DH, 128).astype(f32)
                part = v * jnp.concatenate([p_s[:, c:c + 128]] * (DH // 8), axis=0)
                st['o'] = st['o'] + part if c else part

        def finish():
            st['o'] = jnp.broadcast_to(jnp.sum(st['o'], axis=-1, keepdims=True), (DH, 128))

        tasks = {s: [lambda j=4 * s + i: qk(j) for i in range(4)] for s in range(4)}
        tasks.update({4 + s: [lambda j=4 * s + i: pv(j) for i in range(4)] for s in range(4)})
        tasks[3].append(softmax)
        tasks[7].append(finish)
        return tasks

    def k_iteration(it, feed, tasks=None, last=False):
        iteration(it, 0, lambda s: [kv(int(last), (it + 1) & (H - 1), s)], feed, tasks or {},
                  GAP_IDLE if tasks is None else GAP_BUSY)

    def q_feed(first, n):
        return pieces(parts(wq, wq_b), first, n, w_sem.at[0])

    def gu_feed(it):
        return pieces([(wg, wg_b), (wu, wu_b)], FEED // 2 * (it - IT_GU), FEED // 2, w_sem.at[1])

    small = [pltpu.make_async_copy(x_hbm, x_v, s_sem.at[0]),
             pltpu.make_async_copy(gw_hbm, gw_v, s_sem.at[1]),
             pltpu.make_async_copy(wr_hbm, wr_v, s_sem.at[2])]
    kv(0, 0, 0).start(priority=1)
    for c in small:
        c.start()
    for s in range(1, STEPS):
        kv(0, 0, s).start(priority=1)
    for c in q_feed(0, LEAD // 2):
        c.start(priority=0)
        pl.delay(GAP_BUSY)
    loop(0, IT_GU - 1, lambda it: k_iteration(it, q_feed((LEAD + FEED * it) // 2, FEED // 2)))

    for c in small:
        c.wait()
    a_s[...] = jnp.zeros_like(a_s)
    for c in range(0, D, 128):
        x_c[c:c + 128, :] = _column(x_v[0, :, c:c + 128].astype(f32))
    d_lead = FEED // 4 * (2 * H - 1 - IT_D)
    k_iteration(IT_GU - 1, q_feed((LEAD + FEED * (IT_GU - 1)) // 2, (FEED - LEAD) // 2)
                + pieces(parts(wd, wd_b), d_lead, LEAD // 4, w_sem.at[2]), {})
    k_iteration(IT_GU, gu_feed(IT_GU))
    landed(wq_b, w_sem.at[0])
    landed(wd_b.at[tile_rows(4 * d_lead, LEAD)], w_sem.at[2])
    loop(IT_GU + 1, H - 1, lambda it: k_iteration(
        it, gu_feed(it), {2 * j: q_block(4 * (it - IT_GU - 1) + j) for j in range(4)}))
    k_iteration(H - 1, gu_feed(H - 1), last=True)

    def v_iteration(it, feed, extra, project, nxt=None):
        st = {}
        tasks = attention(it - H, st)
        for s, task in extra:
            tasks[s].append(task)
        if project:
            h = it - IT_PROJ
            tasks[project].append(lambda: proj(0, h, q_c[pl.ds(_mult(h * DH, DH), DH), :]))
            tasks[7].append(lambda: proj(1, h, st['o']))
        else:
            def keep():
                q_c[pl.ds(_mult((it - H) * DH, DH), DH), :] = st['o']
            tasks[7].append(keep)
        iteration(it, 1, nxt or (lambda s: [kv(1, it + 1 - H, s)]), feed, tasks, GAP_BUSY)

    def o_feed(it):
        return pieces(parts(wo, wo_b), FEED // 2 * (it - IT_O), FEED // 2, w_sem.at[3 + (it & 1)])

    def o_landed(it):
        landed(wo_b.at[tile_rows(2 * FEED * (it - IT_O), 2 * FEED)], w_sem.at[3 + (it & 1)])

    def ffn_block(it):
        @pl.when(it == IT_O)
        def _():
            landed(wg_b, w_sem.at[1])
            landed(wu_b, w_sem.at[1])
        pl.when(it > IT_O)(lambda: o_landed(it - 1))
        pl.when(it < IT_O + 6)(lambda: gate_block(it - IT_O))
        pl.when(it >= IT_O + 6)(lambda: up_block(it - IT_O - 6))

    def d_feed(it):
        return pieces(parts(wd, wd_b), FEED // 4 * (it - IT_D), FEED // 4, w_sem.at[3 + (it & 1)])

    def down_block(it):
        landed(wd_b.at[tile_rows(FEED * (it - IT_D), FEED)], w_sem.at[3 + (it & 1)])
        y_s[...] = jnp.concatenate(down(split(y_s[...]), FEED // DT * (it - IT_D), 0, FEED), axis=1)

    def d_block(it):
        @pl.when(it == IT_D)
        def _():
            o_landed(it - 1)
            y_s[...] = jnp.concatenate(down(split(jnp.zeros((8, D), f32)), 0, 4 * d_lead, LEAD), axis=1)
        pl.when(it > IT_D)(lambda: down_block(it - 1))

    loop(H, IT_O, lambda it: v_iteration(it, gu_feed(it), [], None))
    loop(IT_O, IT_PROJ, lambda it: v_iteration(it, o_feed(it), [(5, lambda: ffn_block(it))], None))
    loop(IT_PROJ, IT_D, lambda it: v_iteration(it, o_feed(it), [(4, lambda: o_landed(it - 1))], 5))
    loop(IT_D, 2 * H - 1, lambda it: v_iteration(it, d_feed(it), [(4, lambda: d_block(it))], 5))

    xf = x_v[0].astype(f32)
    gate = jax.nn.sigmoid(jnp.sum(xf * gw_v[...].astype(f32).reshape(1, D), axis=-1, keepdims=True))
    rsel = jax.nn.sigmoid(jnp.sum(xf * wr_v[...].astype(f32).reshape(1, D), axis=-1, keepdims=True))

    it = 2 * H - 1
    first = 4 * d_lead + LEAD
    rest = []
    for j in range(4):
        t = first + LAST
        for n in (TAIL if j == 3 else (sum(TAIL),)):
            rows = pl.ds(8 * t, 8 * n)
            rest.append((j, t, n, pltpu.make_async_copy(wd.at[j, rows], wd_b.at[j, rows], e_sem.at[len(rest)])))
            t += n
        assert 8 * t == wd.shape[1]
    v_iteration(it, pieces(parts(wd, wd_b), first // 4, LAST // 4, w_sem.at[3 + (it & 1)]),
                [(2, lambda: down_block(it - 1))], 1, lambda s: [] if s else [c[3] for c in rest])

    landed(wd_b.at[tile_rows(first, LAST)], w_sem.at[3 + (it & 1)])
    a = jnp.sum(a_s[...], axis=0, keepdims=True)
    y = down(split(y_s[...]), 0, first, LAST)
    for j, t, n, c in rest:
        c.wait()
        y = down(y, 0, t, n, (j,))
    y = jnp.sum(jnp.concatenate(y, axis=1), axis=0, keepdims=True)
    b = xf + (xf * 0.0 + y * rsel)
    out_ref[0] = (gate * a + (1.0 - gate) * b).astype(bf16)


def _tile_list(w):
    r, c = w.shape
    return w.reshape(r // 8, 8, c // 128, 128).transpose(0, 2, 1, 3).reshape(-1, 128)


@jax.jit
def pallas_gated_mix__sliding_block_cached__moe_arch_mod__decode_kernel(
        A_x, A_k_cache, A_v_cache, A_wq, A_wo, B_x, B_w_r, B_w_gate, B_w_up, B_w_down, gate_w):
    del B_x
    kT = jnp.swapaxes(A_k_cache, 2, 3).reshape(H, DH // 16, 16, SK)
    vT = jnp.swapaxes(A_v_cache, 2, 3).reshape(H, DH // 16, 16, SK)
    wg, wu = _tile_list(B_w_gate), _tile_list(B_w_up)
    wq, wo = _tile_list(A_wq).reshape(2, -1, 128), _tile_list(A_wo).reshape(2, -1, 128)
    wd = _tile_list(B_w_down).reshape(4, -1, 128)
    vmem = pltpu.VMEM
    dma = pltpu.SemaphoreType.DMA
    return pl.pallas_call(
        _kernel,
        out_shape=jax.ShapeDtypeStruct((1, 1, D), bf16),
        in_specs=[pl.BlockSpec(memory_space=pl.ANY)] * 10,
        out_specs=pl.BlockSpec(memory_space=pltpu.VMEM),
        scratch_shapes=[
            vmem((1, 1, D), bf16), vmem((D,), bf16), vmem((D,), bf16),
            vmem(wq.shape, bf16), vmem((H, DH // 16, 16, W), bf16), vmem((RING, DH // 16, 16, W), bf16),
            vmem(wo.shape, bf16), vmem(wg.shape, bf16), vmem(wu.shape, bf16), vmem(wd.shape, bf16),
            vmem((D, 128), f32), vmem((H * DH, 128), f32), vmem((F, 128), f32),
            vmem((8, W), f32), vmem((8, D), f32), vmem((8, D), f32),
            dma((STEPS,)), dma((5,)), dma((3,)), dma((3 + len(TAIL),)),
        ],
        compiler_params=pltpu.CompilerParams(
            vmem_limit_bytes=100 * 1024 * 1024,
            disable_semaphore_checks=True,
            disable_bounds_checks=True,
        ),
        name="gated_mix_decode",
    )(A_x, kT, vT, wq, wo, B_w_r, wg, wu, wd, gate_w)
```

```python
import jax
import jax.numpy as jnp
import jax.experimental.pallas as pl
import jax.experimental.pallas.tpu as pltpu

H, DH, SK, D, F = 32, 192, 32768, 640, 1536
W = min(4096, max(256, SK // 4))
BASE = SK - W
DT = D // 128

STEPS = 8
RING = 4
PIECE = 32
FEED = 40
LEAD = 32
LAST = 24
TAIL = (24, 16, 12, 8, 4)
GAP_IDLE = 58
GAP_BUSY = 30
IT_GU, IT_O, IT_D = 24, 36, 60
IT_PROJ = 2 * H - H // 2

f32 = jnp.float32
bf16 = jnp.bfloat16


def _mult(i, n):
    return i if isinstance(i, int) else pl.multiple_of(i, n)


def _column(row):
    return jnp.broadcast_to(row, (128, 128)).T


def _tiles(ref, first, n):
    out = []
    for i in range(0, n, 2):
        w = ref[pl.ds(_mult(8 * (first + i), 16), 16), :].astype(f32)
        out += [w[:8], w[8:]]
    return out


def _kernel(x_hbm, kT, vT, wq, wo, wr_hbm, wg, wu, wd, gw_hbm, out_ref,
            x_v, wr_v, gw_v, wq_b, k_b, v_b, wo_b, wg_b, wu_b, wd_b,
            x_c, q_c, h_c, p_s, a_s, g_s, kv_sem, w_sem, s_sem, e_sem):
    def kv(which, h, s):
        rows, c = pl.ds(8 * (s // 4), 8), (W // 4) * (3 - s if s < 4 else s - 4)
        src = (kT, vT)[which].at[h, :, rows, pl.ds(BASE + c, W // 4)]
        dst = k_b.at[h] if which == 0 else v_b.at[h & (RING - 1)]
        return pltpu.make_async_copy(src, dst.at[:, rows, pl.ds(c, W // 4)], kv_sem.at[s])

    def pieces(parts, first, n, sem):
        out = []
        for i in range(0, n, 2):
            for src, dst in parts:
                for p in (first + i, first + i + 1):
                    rows = pl.ds(_mult(p * PIECE, PIECE), PIECE)
                    out.append(pltpu.make_async_copy(src.at[rows], dst.at[rows], sem))
        return out

    def parts(src, dst):
        return [(src.at[j], dst.at[j]) for j in range(src.shape[0])]

    def tile_rows(first, n):
        return (slice(None), pl.ds(_mult(8 * first, 8), 8 * n))

    def landed(buf, sem):
        pltpu.make_async_copy(buf, buf, sem).wait()

    def iteration(it, which, nxt, feed, tasks, gap):
        for s in range(STEPS):
            kv(which, it & (H - 1), s).wait()
            for c in nxt(s):
                c.start(priority=1)
            todo = list(tasks.get(s, []))
            for i, c in enumerate(feed[s * FEED // STEPS:(s + 1) * FEED // STEPS]):
                if i and todo:
                    pl.delay(1)
                    todo.pop(0)()
                    pl.delay(1)
                elif i:
                    pl.delay(gap)
                c.start(priority=0)
            for task in todo:
                task()

    def loop(lo, hi, fn):
        jax.lax.fori_loop(lo, hi, lambda i, c: fn(i), None)

    def x_dot(w_refs, width, b, acc, n):
        def part(k):
            for rt in range(k * (D // 8) // n, (k + 1) * (D // 8) // n):
                xc = x_c[8 * rt:8 * rt + 8, :]
                j, r = divmod(rt, D // 8 // len(w_refs))
                p = [w * xc for w in _tiles(w_refs[j], r * width + 2 * b, 2)]
                acc[:] = [u + v for u, v in zip(acc, p)] if rt else p
        return [lambda k=k: part(k) for k in range(n)]

    def q_block(b):
        q = []

        def store():
            for i in range(2):
                q_c[pl.ds(_mult((2 * b + i) * 128, 128), 128), :] = _column(jnp.sum(q[i], axis=0, keepdims=True))
        return x_dot([wq_b.at[0], wq_b.at[1]], H * DH // 128, b, q, 4) + [store]

    def gate_block(b):
        g = []
        x_dot([wg_b], F // 128, b, g, 1)[0]()
        for i in range(2):
            h_c[pl.ds(_mult((2 * b + i) * 128, 128), 8), :] = jnp.broadcast_to(
                jax.nn.silu(jnp.sum(g[i], axis=0, keepdims=True)), (8, 128)) * g_s[1]

    def up_block(b):
        u = []
        x_dot([wu_b], F // 128, b, u, 1)[0]()
        for i in range(2):
            r = _mult((2 * b + i) * 128, 128)
            h_c[pl.ds(r, 128), :] = _column(h_c[pl.ds(r, 8), :][:1] * jnp.sum(u[i], axis=0, keepdims=True))

    def split(a):
        return [a[:, c:c + 128] for c in range(0, D, 128)]

    def proj(half, h, o):
        acc = split(a_s[...])
        for t, w in enumerate(_tiles(wo_b.at[half], h * (DH // 8 * DT), DH // 8 * DT)):
            acc[t % DT] = acc[t % DT] + w * o[8 * (t // DT):8 * (t // DT) + 8]
        a_s[...] = jnp.concatenate(acc, axis=1)

    def down(acc, rt, first, n, quarters=range(4)):
        for j in quarters:
            for t, w in enumerate(_tiles(wd_b.at[j], DT * rt + first, n), first):
                rows = pl.ds(_mult(j * (F // 4) + 8 * (rt + t // DT), 8), 8)
                acc[t % DT] = acc[t % DT] + w * h_c[rows, :]
        return acc

    def attention(h, st):
        head = pl.ds(_mult(h * DH, DH), DH)

        def qk(j):
            q = q_c[head, :]
            for c in range(256 * j, 256 * (j + 1), 128):
                k = k_b[h, :, :, c:c + 128].reshape(DH, 128).astype(f32)
                p_s[:, c:c + 128] = jnp.broadcast_to(jnp.sum(k * q, axis=0, keepdims=True), (8, 128))

        def softmax():
            s = p_s[...] * (DH ** -0.5)
            e = jnp.exp(s - jnp.max(s, axis=-1, keepdims=True))
            p_s[...] = e * (g_s[0][:, :1] / jnp.sum(e, axis=-1, keepdims=True))

        def pv(j):
            for c in range(256 * j, 256 * (j + 1), 128):
                v = v_b[h & (RING - 1), :, :, c:c + 128].reshape(DH, 128).astype(f32)
                part = v * jnp.concatenate([p_s[:, c:c + 128]] * (DH // 8), axis=0)
                st['o'] = st['o'] + part if c else part

        def finish():
            st['o'] = jnp.broadcast_to(jnp.sum(st['o'], axis=-1, keepdims=True), (DH, 128))

        tasks = {s: [lambda j=4 * s + i: qk(j) for i in range(4)] for s in range(4)}
        tasks.update({4 + s: [lambda j=4 * s + i: pv(j) for i in range(4)] for s in range(4)})
        tasks[3].append(softmax)
        tasks[7].append(finish)
        return tasks

    def k_iteration(it, feed, tasks=None, last=False):
        iteration(it, 0, lambda s: [kv(int(last), (it + 1) & (H - 1), s)], feed, tasks or {},
                  GAP_IDLE if tasks is None else GAP_BUSY)

    def q_feed(first, n):
        return pieces(parts(wq, wq_b), first, n, w_sem.at[0])

    def gu_feed(it):
        return pieces([(wg, wg_b), (wu, wu_b)], FEED // 2 * (it - IT_GU), FEED // 2, w_sem.at[1])

    small = [pltpu.make_async_copy(x_hbm, x_v, s_sem.at[0]),
             pltpu.make_async_copy(gw_hbm, gw_v, s_sem.at[1]),
             pltpu.make_async_copy(wr_hbm, wr_v, s_sem.at[2])]
    kv(0, 0, 0).start(priority=1)
    for c in small:
        c.start()
    for s in range(1, STEPS):
        kv(0, 0, s).start(priority=1)
    for c in q_feed(0, LEAD // 2):
        c.start(priority=0)
        pl.delay(GAP_BUSY)
    loop(0, IT_GU - 1, lambda it: k_iteration(it, q_feed((LEAD + FEED * it) // 2, FEED // 2)))

    for c in small:
        c.wait()
    xf = x_v[0].astype(f32)
    gate = jax.nn.sigmoid(jnp.sum(xf * gw_v[...].astype(f32).reshape(1, D), axis=-1, keepdims=True))
    rsel = jax.nn.sigmoid(jnp.sum(xf * wr_v[...].astype(f32).reshape(1, D), axis=-1, keepdims=True))
    g_s[0] = jnp.broadcast_to(gate, (8, 128))
    g_s[1] = jnp.broadcast_to((1.0 - gate) * rsel, (8, 128))
    a_s[...] = jnp.where(jax.lax.broadcasted_iota(jnp.int32, (8, D), 0) == 0, (1.0 - gate) * (xf + xf * 0.0), 0.0)
    for c in range(0, D, 128):
        x_c[c:c + 128, :] = _column(x_v[0, :, c:c + 128].astype(f32))
    d_lead = FEED // 4 * (2 * H - 1 - IT_D)
    k_iteration(IT_GU - 1, q_feed((LEAD + FEED * (IT_GU - 1)) // 2, (FEED - LEAD) // 2)
                + pieces(parts(wd, wd_b), d_lead, LEAD // 4, w_sem.at[2]), {})
    k_iteration(IT_GU, gu_feed(IT_GU))
    landed(wq_b, w_sem.at[0])
    landed(wd_b.at[tile_rows(4 * d_lead, LEAD)], w_sem.at[2])
    loop(IT_GU + 1, H - 1, lambda it: k_iteration(
        it, gu_feed(it), {2 * j: q_block(4 * (it - IT_GU - 1) + j) for j in range(4)}))
    k_iteration(H - 1, gu_feed(H - 1), last=True)

    def v_iteration(it, feed, extra, project, nxt=None):
        st = {}
        tasks = attention(it - H, st)
        for s, task in extra:
            tasks[s].append(task)
        if project:
            h = it - IT_PROJ
            tasks[project].append(lambda: proj(0, h, q_c[pl.ds(_mult(h * DH, DH), DH), :]))
            tasks[7].append(lambda: proj(1, h, st['o']))
        else:
            def keep():
                q_c[pl.ds(_mult((it - H) * DH, DH), DH), :] = st['o']
            tasks[7].append(keep)
        iteration(it, 1, nxt or (lambda s: [kv(1, it + 1 - H, s)]), feed, tasks, GAP_BUSY)

    def o_feed(it):
        return pieces(parts(wo, wo_b), FEED // 2 * (it - IT_O), FEED // 2, w_sem.at[3 + (it & 1)])

    def o_landed(it):
        landed(wo_b.at[tile_rows(2 * FEED * (it - IT_O), 2 * FEED)], w_sem.at[3 + (it & 1)])

    def ffn_block(it):
        @pl.when(it == IT_O)
        def _():
            landed(wg_b, w_sem.at[1])
            landed(wu_b, w_sem.at[1])
        pl.when(it > IT_O)(lambda: o_landed(it - 1))
        pl.when(it < IT_O + 6)(lambda: gate_block(it - IT_O))
        pl.when(it >= IT_O + 6)(lambda: up_block(it - IT_O - 6))

    def d_feed(it):
        return pieces(parts(wd, wd_b), FEED // 4 * (it - IT_D), FEED // 4, w_sem.at[3 + (it & 1)])

    def down_block(it):
        landed(wd_b.at[tile_rows(FEED * (it - IT_D), FEED)], w_sem.at[3 + (it & 1)])
        a_s[...] = jnp.concatenate(down(split(a_s[...]), FEED // DT * (it - IT_D), 0, FEED), axis=1)

    def d_block(it):
        @pl.when(it == IT_D)
        def _():
            o_landed(it - 1)
            a_s[...] = jnp.concatenate(down(split(a_s[...]), 0, 4 * d_lead, LEAD), axis=1)
        pl.when(it > IT_D)(lambda: down_block(it - 1))

    loop(H, IT_O, lambda it: v_iteration(it, gu_feed(it), [], None))
    loop(IT_O, IT_PROJ, lambda it: v_iteration(it, o_feed(it), [(5, lambda: ffn_block(it))], None))
    loop(IT_PROJ, IT_D, lambda it: v_iteration(it, o_feed(it), [(4, lambda: o_landed(it - 1))], 5))
    loop(IT_D, 2 * H - 1, lambda it: v_iteration(it, d_feed(it), [(4, lambda: d_block(it))], 5))

    it = 2 * H - 1
    first = 4 * d_lead + LEAD
    rest = []
    for j in range(4):
        t = first + LAST
        for n in (TAIL if j == 3 else (sum(TAIL),)):
            rows = pl.ds(8 * t, 8 * n)
            rest.append((j, t, n, pltpu.make_async_copy(wd.at[j, rows], wd_b.at[j, rows], e_sem.at[len(rest)])))
            t += n
        assert 8 * t == wd.shape[1]
    v_iteration(it, pieces(parts(wd, wd_b), first // 4, LAST // 4, w_sem.at[3 + (it & 1)]),
                [(2, lambda: down_block(it - 1))], 1, lambda s: [] if s else [c[3] for c in rest])

    landed(wd_b.at[tile_rows(first, LAST)], w_sem.at[3 + (it & 1)])
    acc = down(split(a_s[...]), 0, first, LAST)
    for j, t, n, c in rest:
        c.wait()
        acc = down(acc, 0, t, n, (j,))
    out_ref[0] = jnp.sum(jnp.concatenate(acc, axis=1), axis=0, keepdims=True).astype(bf16)


def _tile_list(w):
    r, c = w.shape
    return w.reshape(r // 8, 8, c // 128, 128).transpose(0, 2, 1, 3).reshape(-1, 128)


@jax.jit
def pallas_gated_mix__sliding_block_cached__moe_arch_mod__decode_kernel(
        A_x, A_k_cache, A_v_cache, A_wq, A_wo, B_x, B_w_r, B_w_gate, B_w_up, B_w_down, gate_w):
    del B_x
    kT = jnp.swapaxes(A_k_cache, 2, 3).reshape(H, DH // 16, 16, SK)
    vT = jnp.swapaxes(A_v_cache, 2, 3).reshape(H, DH // 16, 16, SK)
    wg, wu = _tile_list(B_w_gate), _tile_list(B_w_up)
    wq, wo = _tile_list(A_wq).reshape(2, -1, 128), _tile_list(A_wo).reshape(2, -1, 128)
    wd = _tile_list(B_w_down).reshape(4, -1, 128)
    vmem = pltpu.VMEM
    dma = pltpu.SemaphoreType.DMA
    return pl.pallas_call(
        _kernel,
        out_shape=jax.ShapeDtypeStruct((1, 1, D), bf16),
        in_specs=[pl.BlockSpec(memory_space=pl.ANY)] * 10,
        out_specs=pl.BlockSpec(memory_space=pltpu.VMEM),
        scratch_shapes=[
            vmem((1, 1, D), bf16), vmem((D,), bf16), vmem((D,), bf16),
            vmem(wq.shape, bf16), vmem((H, DH // 16, 16, W), bf16), vmem((RING, DH // 16, 16, W), bf16),
            vmem(wo.shape, bf16), vmem(wg.shape, bf16), vmem(wu.shape, bf16), vmem(wd.shape, bf16),
            vmem((D, 128), f32), vmem((H * DH, 128), f32), vmem((F, 128), f32),
            vmem((8, W), f32), vmem((8, D), f32), vmem((2, 8, 128), f32),
            dma((STEPS,)), dma((5,)), dma((3,)), dma((3 + len(TAIL),)),
        ],
        compiler_params=pltpu.CompilerParams(
            vmem_limit_bytes=100 * 1024 * 1024,
            disable_semaphore_checks=True,
            disable_bounds_checks=True,
        ),
        name="gated_mix_decode",
    )(A_x, kT, vT, wq, wo, B_w_r, wg, wu, wd, gate_w)
```

```python
import jax
import jax.numpy as jnp
import jax.experimental.pallas as pl
import jax.experimental.pallas.tpu as pltpu

H, DH, SK, D, F = 32, 192, 32768, 640, 1536
W = min(4096, max(256, SK // 4))
BASE = SK - W
DT = D // 128

STEPS = 8
RING = 4
PIECE = 32
FEED = 40
LEAD = 32
LAST = 24
TAIL = (24, 16, 12, 8, 4)
GAP_IDLE = 58
GAP_BUSY = 30
IT_GU, IT_O, IT_D = 24, 36, 60
IT_PROJ = 2 * H - H // 2

f32 = jnp.float32
bf16 = jnp.bfloat16


def _mult(i, n):
    return i if isinstance(i, int) else pl.multiple_of(i, n)


def _column(row):
    return jnp.broadcast_to(row, (128, 128)).T


def _tiles(ref, first, n):
    out = []
    for i in range(0, n, 2):
        w = ref[pl.ds(_mult(8 * (first + i), 16), 16), :].astype(f32)
        out += [w[:8], w[8:]]
    return out


def _kernel(x_hbm, kT, vT, wq, wo, wr_hbm, wg, wu, wd, gw_hbm, out_ref,
            x_v, wr_v, gw_v, wq_b, k_b, v_b, wo_b, wg_b, wu_b, wd_b,
            x_c, q_c, h_c, p_s, a_s, g_s, kv_sem, w_sem, s_sem, e_sem):
    def kv(which, h, s):
        rows, c = pl.ds(8 * (s // 4), 8), (W // 4) * (3 - s if s < 4 else s - 4)
        src = (kT, vT)[which].at[h, :, rows, pl.ds(BASE + c, W // 4)]
        dst = k_b.at[h] if which == 0 else v_b.at[h & (RING - 1)]
        return pltpu.make_async_copy(src, dst.at[:, rows, pl.ds(c, W // 4)], kv_sem.at[s])

    def pieces(parts, first, n):
        out = []
        for i in range(0, n, 2):
            for src, dst, sem in parts:
                for p in (first + i, first + i + 1):
                    rows = pl.ds(_mult(p * PIECE, PIECE), PIECE)
                    out.append(pltpu.make_async_copy(src.at[rows], dst.at[rows], sem))
        return out

    def parts(src, dst, sem):
        return [(src.at[j], dst.at[j], sem) for j in range(src.shape[0])]

    def tile_rows(first, n):
        return (slice(None), pl.ds(_mult(8 * first, 8), 8 * n))

    def landed(buf, sem):
        pltpu.make_async_copy(buf, buf, sem).wait()

    def iteration(it, which, nxt, feed, tasks, gap):
        for s in range(STEPS):
            kv(which, it & (H - 1), s).wait()
            for c in nxt(s):
                c.start(priority=1)
            todo = list(tasks.get(s, []))
            for i, c in enumerate(feed[s * FEED // STEPS:(s + 1) * FEED // STEPS]):
                if i and todo:
                    pl.delay(1)
                    todo.pop(0)()
                    pl.delay(1)
                elif i:
                    pl.delay(gap)
                c.start(priority=0)
            for task in todo:
                task()

    def loop(lo, hi, fn):
        jax.lax.fori_loop(lo, hi, lambda i, c: fn(i), None)

    def x_dot(w_refs, width, b, acc, n):
        def part(k):
            for rt in range(k * (D // 8) // n, (k + 1) * (D // 8) // n):
                xc = x_c[8 * rt:8 * rt + 8, :]
                j, r = divmod(rt, D // 8 // len(w_refs))
                p = [w * xc for w in _tiles(w_refs[j], r * width + 2 * b, 2)]
                acc[:] = [u + v for u, v in zip(acc, p)] if rt else p
        return [lambda k=k: part(k) for k in range(n)]

    def q_block(b):
        q = []

        def store():
            for i in range(2):
                q_c[pl.ds(_mult((2 * b + i) * 128, 128), 128), :] = _column(jnp.sum(q[i], axis=0, keepdims=True))
        return x_dot([wq_b.at[0], wq_b.at[1]], H * DH // 128, b, q, 4) + [store]

    def gate_block(b):
        g = []
        x_dot([wg_b], F // 128, b, g, 1)[0]()
        for i in range(2):
            h_c[pl.ds(_mult((2 * b + i) * 128, 128), 8), :] = jnp.broadcast_to(
                jax.nn.silu(jnp.sum(g[i], axis=0, keepdims=True)), (8, 128)) * g_s[1]

    def up_block(b):
        u = []
        x_dot([wu_b], F // 128, b, u, 1)[0]()
        for i in range(2):
            r = _mult((2 * b + i) * 128, 128)
            h_c[pl.ds(r, 128), :] = _column(h_c[pl.ds(r, 8), :][:1] * jnp.sum(u[i], axis=0, keepdims=True))

    def split(a):
        return [a[:, c:c + 128] for c in range(0, D, 128)]

    def proj(half, h, o):
        acc = split(a_s[...])
        for t, w in enumerate(_tiles(wo_b.at[half], h * (DH // 8 * DT), DH // 8 * DT)):
            acc[t % DT] = acc[t % DT] + w * o[8 * (t // DT):8 * (t // DT) + 8]
        a_s[...] = jnp.concatenate(acc, axis=1)

    def down(acc, rt, first, n, quarters=range(4)):
        for j in quarters:
            for t, w in enumerate(_tiles(wd_b.at[j], DT * rt + first, n), first):
                rows = pl.ds(_mult(j * (F // 4) + 8 * (rt + t // DT), 8), 8)
                acc[t % DT] = acc[t % DT] + w * h_c[rows, :]
        return acc

    def attention(h, st):
        head = pl.ds(_mult(h * DH, DH), DH)

        def qk(j):
            q = q_c[head, :]
            for c in range(256 * j, 256 * (j + 1), 128):
                k = k_b[h, :, :, c:c + 128].reshape(DH, 128).astype(f32)
                p_s[:, c:c + 128] = jnp.broadcast_to(jnp.sum(k * q, axis=0, keepdims=True), (8, 128))

        def softmax():
            s = p_s[...] * (DH ** -0.5)
            e = jnp.exp(s - jnp.max(s, axis=-1, keepdims=True))
            p_s[...] = e * (g_s[0][:, :1] / jnp.sum(e, axis=-1, keepdims=True))

        def pv(j):
            for c in range(256 * j, 256 * (j + 1), 128):
                v = v_b[h & (RING - 1), :, :, c:c + 128].reshape(DH, 128).astype(f32)
                part = v * jnp.concatenate([p_s[:, c:c + 128]] * (DH // 8), axis=0)
                st['o'] = st['o'] + part if c else part

        def finish():
            st['o'] = jnp.broadcast_to(jnp.sum(st['o'], axis=-1, keepdims=True), (DH, 128))

        tasks = {s: [lambda j=4 * s + i: qk(j) for i in range(4)] for s in range(4)}
        tasks.update({4 + s: [lambda j=4 * s + i: pv(j) for i in range(4)] for s in range(4)})
        tasks[3].append(softmax)
        tasks[7].append(finish)
        return tasks

    def k_iteration(it, feed, tasks=None, last=False):
        iteration(it, 0, lambda s: [kv(int(last), (it + 1) & (H - 1), s)], feed, tasks or {},
                  GAP_IDLE if tasks is None else GAP_BUSY)

    def q_feed(first, n):
        return pieces(parts(wq, wq_b, w_sem.at[0]), first, n)

    def gu_feed(it):
        return pieces([(wg, wg_b, w_sem.at[1]), (wu, wu_b, w_sem.at[2])], FEED // 2 * (it - IT_GU), FEED // 2)

    small = [pltpu.make_async_copy(x_hbm, x_v, s_sem.at[0]),
             pltpu.make_async_copy(gw_hbm, gw_v, s_sem.at[1]),
             pltpu.make_async_copy(wr_hbm, wr_v, s_sem.at[2])]
    kv(0, 0, 0).start(priority=1)
    for c in small:
        c.start()
    for s in range(1, STEPS):
        kv(0, 0, s).start(priority=1)
    for c in q_feed(0, LEAD // 2):
        c.start(priority=0)
        pl.delay(GAP_BUSY)
    loop(0, IT_GU - 1, lambda it: k_iteration(it, q_feed((LEAD + FEED * it) // 2, FEED // 2)))

    for c in small:
        c.wait()
    xf = x_v[0].astype(f32)
    gate = jax.nn.sigmoid(jnp.sum(xf * gw_v[...].astype(f32).reshape(1, D), axis=-1, keepdims=True))
    rsel = jax.nn.sigmoid(jnp.sum(xf * wr_v[...].astype(f32).reshape(1, D), axis=-1, keepdims=True))
    g_s[0] = jnp.broadcast_to(gate, (8, 128))
    g_s[1] = jnp.broadcast_to((1.0 - gate) * rsel, (8, 128))
    a_s[...] = jnp.where(jax.lax.broadcasted_iota(jnp.int32, (8, D), 0) == 0, (1.0 - gate) * (xf + xf * 0.0), 0.0)
    for c in range(0, D, 128):
        x_c[c:c + 128, :] = _column(x_v[0, :, c:c + 128].astype(f32))
    d_lead = FEED // 4 * (2 * H - 1 - IT_D)
    k_iteration(IT_GU - 1, q_feed((LEAD + FEED * (IT_GU - 1)) // 2, (FEED - LEAD) // 2)
                + pieces(parts(wd, wd_b, w_sem.at[3]), d_lead, LEAD // 4), {})
    k_iteration(IT_GU, gu_feed(IT_GU))
    landed(wq_b, w_sem.at[0])
    landed(wd_b.at[tile_rows(4 * d_lead, LEAD)], w_sem.at[3])
    loop(IT_GU + 1, H - 1, lambda it: k_iteration(
        it, gu_feed(it), {2 * j: q_block(4 * (it - IT_GU - 1) + j) for j in range(4)}))
    k_iteration(H - 1, gu_feed(H - 1), last=True)

    def v_iteration(it, feed, extra, project, nxt=None):
        st = {}
        tasks = attention(it - H, st)
        for s, task in extra:
            tasks[s].append(task)
        if project:
            h = it - IT_PROJ
            tasks[project].append(lambda: proj(0, h, q_c[pl.ds(_mult(h * DH, DH), DH), :]))
            tasks[7].append(lambda: proj(1, h, st['o']))
        else:
            def keep():
                q_c[pl.ds(_mult((it - H) * DH, DH), DH), :] = st['o']
            tasks[7].append(keep)
        iteration(it, 1, nxt or (lambda s: [kv(1, it + 1 - H, s)]), feed, tasks, GAP_BUSY)

    def o_feed(it):
        return pieces(parts(wo, wo_b, w_sem.at[3 + (it & 1)]), FEED // 2 * (it - IT_O), FEED // 2)

    def o_landed(it):
        landed(wo_b.at[tile_rows(2 * FEED * (it - IT_O), 2 * FEED)], w_sem.at[3 + (it & 1)])

    def ffn_block(it):
        @pl.when(it == IT_O)
        def _():
            landed(wg_b, w_sem.at[1])
            landed(wu_b, w_sem.at[2])
        pl.when(it > IT_O)(lambda: o_landed(it - 1))
        pl.when(it < IT_O + 6)(lambda: gate_block(it - IT_O))
        pl.when(it >= IT_O + 6)(lambda: up_block(it - IT_O - 6))

    def d_feed(it):
        return pieces(parts(wd, wd_b, w_sem.at[3 + (it & 1)]), FEED // 4 * (it - IT_D), FEED // 4)

    def down_block(it):
        landed(wd_b.at[tile_rows(FEED * (it - IT_D), FEED)], w_sem.at[3 + (it & 1)])
        a_s[...] = jnp.concatenate(down(split(a_s[...]), FEED // DT * (it - IT_D), 0, FEED), axis=1)

    def d_block(it):
        @pl.when(it == IT_D)
        def _():
            o_landed(it - 1)
            a_s[...] = jnp.concatenate(down(split(a_s[...]), 0, 4 * d_lead, LEAD), axis=1)
        pl.when(it > IT_D)(lambda: down_block(it - 1))

    loop(H, IT_O, lambda it: v_iteration(it, gu_feed(it), [], None))
    loop(IT_O, IT_PROJ, lambda it: v_iteration(it, o_feed(it), [(5, lambda: ffn_block(it))], None))
    loop(IT_PROJ, IT_D, lambda it: v_iteration(it, o_feed(it), [(4, lambda: o_landed(it - 1))], 5))
    loop(IT_D, 2 * H - 1, lambda it: v_iteration(it, d_feed(it), [(4, lambda: d_block(it))], 5))

    it = 2 * H - 1
    first = 4 * d_lead + LEAD
    rest = []
    for j in range(4):
        t = first + LAST
        for n in (TAIL if j == 3 else (sum(TAIL),)):
            rows = pl.ds(8 * t, 8 * n)
            rest.append((j, t, n, pltpu.make_async_copy(wd.at[j, rows], wd_b.at[j, rows], e_sem.at[len(rest)])))
            t += n
        assert 8 * t == wd.shape[1]
    v_iteration(it, pieces(parts(wd, wd_b, w_sem.at[3 + (it & 1)]), first // 4, LAST // 4),
                [(2, lambda: down_block(it - 1))], 1, lambda s: [] if s else [c[3] for c in rest])

    landed(wd_b.at[tile_rows(first, LAST)], w_sem.at[3 + (it & 1)])
    acc = down(split(a_s[...]), 0, first, LAST)
    for j, t, n, c in rest:
        c.wait()
        acc = down(acc, 0, t, n, (j,))
    out_ref[0] = jnp.sum(jnp.concatenate(acc, axis=1), axis=0, keepdims=True).astype(bf16)


def _tile_list(w):
    r, c = w.shape
    return w.reshape(r // 8, 8, c // 128, 128).transpose(0, 2, 1, 3).reshape(-1, 128)


@jax.jit
def pallas_gated_mix__sliding_block_cached__moe_arch_mod__decode_kernel(
        A_x, A_k_cache, A_v_cache, A_wq, A_wo, B_x, B_w_r, B_w_gate, B_w_up, B_w_down, gate_w):
    del B_x
    kT = jnp.swapaxes(A_k_cache, 2, 3).reshape(H, DH // 16, 16, SK)
    vT = jnp.swapaxes(A_v_cache, 2, 3).reshape(H, DH // 16, 16, SK)
    wg, wu = _tile_list(B_w_gate), _tile_list(B_w_up)
    wq, wo = _tile_list(A_wq).reshape(2, -1, 128), _tile_list(A_wo).reshape(2, -1, 128)
    wd = _tile_list(B_w_down).reshape(4, -1, 128)
    vmem = pltpu.VMEM
    dma = pltpu.SemaphoreType.DMA
    return pl.pallas_call(
        _kernel,
        out_shape=jax.ShapeDtypeStruct((1, 1, D), bf16),
        in_specs=[pl.BlockSpec(memory_space=pl.ANY)] * 10,
        out_specs=pl.BlockSpec(memory_space=pltpu.VMEM),
        scratch_shapes=[
            vmem((1, 1, D), bf16), vmem((D,), bf16), vmem((D,), bf16),
            vmem(wq.shape, bf16), vmem((H, DH // 16, 16, W), bf16), vmem((RING, DH // 16, 16, W), bf16),
            vmem(wo.shape, bf16), vmem(wg.shape, bf16), vmem(wu.shape, bf16), vmem(wd.shape, bf16),
            vmem((D, 128), f32), vmem((H * DH, 128), f32), vmem((F, 128), f32),
            vmem((8, W), f32), vmem((8, D), f32), vmem((2, 8, 128), f32),
            dma((STEPS,)), dma((5,)), dma((3,)), dma((3 + len(TAIL),)),
        ],
        compiler_params=pltpu.CompilerParams(
            vmem_limit_bytes=100 * 1024 * 1024,
            disable_semaphore_checks=True,
            disable_bounds_checks=True,
        ),
        name="gated_mix_decode",
    )(A_x, kT, vT, wq, wo, B_w_r, wg, wu, wd, gate_w)
```

```python
import jax
import jax.numpy as jnp
import jax.experimental.pallas as pl
import jax.experimental.pallas.tpu as pltpu

H, DH, SK, D, F = 32, 192, 32768, 640, 1536
W = min(4096, max(256, SK // 4))
BASE = SK - W
DT = D // 128

STEPS = 8
RING = 4
PIECE = 32
FEED = 40
LEAD = 32
LAST = 24
TAIL = (24, 16, 12, 8, 4)
GAP_IDLE = 58
GAP_BUSY = 30
IT_GU, IT_O, IT_D = 24, 36, 60
IT_PROJ = 2 * H - H // 2

f32 = jnp.float32
bf16 = jnp.bfloat16


def _mult(i, n):
    return i if isinstance(i, int) else pl.multiple_of(i, n)


def _column(row):
    return jnp.broadcast_to(row, (128, 128)).T


def _tiles(ref, first, n):
    out = []
    for i in range(0, n, 2):
        w = ref[pl.ds(_mult(8 * (first + i), 16), 16), :].astype(f32)
        out += [w[:8], w[8:]]
    return out


def _kernel(x_hbm, kT, vT, wq, wo, wr_hbm, wg, wu, wd, gw_hbm, out_ref,
            x_v, wr_v, gw_v, wq_b, k_b, v_b, wo_b, wg_b, wu_b, wd_b,
            x_c, q_c, h_c, p_s, a_s, g_s, kv_sem, w_sem, s_sem, e_sem):
    def kv(which, h, s):
        rows, c = pl.ds(8 * (s // 4), 8), (W // 4) * (3 - s if s < 4 else s - 4)
        src = (kT, vT)[which].at[h, :, rows, pl.ds(BASE + c, W // 4)]
        dst = k_b.at[h] if which == 0 else v_b.at[h & (RING - 1)]
        return pltpu.make_async_copy(src, dst.at[:, rows, pl.ds(c, W // 4)], kv_sem.at[s])

    def pieces(parts, first, n):
        out = []
        for i in range(0, n, 2):
            for src, dst, sem in parts:
                for p in (first + i, first + i + 1):
                    rows = pl.ds(_mult(p * PIECE, PIECE), PIECE)
                    out.append(pltpu.make_async_copy(src.at[rows], dst.at[rows], sem))
        return out

    def parts(src, dst, sem):
        return [(src.at[j], dst.at[j], sem) for j in range(src.shape[0])]

    def tile_rows(first, n):
        return (slice(None), pl.ds(_mult(8 * first, 8), 8 * n))

    def landed(buf, sem):
        pltpu.make_async_copy(buf, buf, sem).wait()

    def iteration(it, which, nxt, feed, tasks, gap):
        for s in range(STEPS):
            kv(which, it & (H - 1), s).wait()
            for c in nxt(s):
                c.start(priority=1)
            todo = list(tasks.get(s, []))
            for i, c in enumerate(feed[s * FEED // STEPS:(s + 1) * FEED // STEPS]):
                if i and todo:
                    pl.delay(1)
                    todo.pop(0)()
                    pl.delay(1)
                elif i:
                    pl.delay(gap)
                c.start(priority=0)
            for task in todo:
                task()

    def loop(lo, hi, fn):
        jax.lax.fori_loop(lo, hi, lambda i, c: fn(i), None)

    def x_dot(w_refs, width, b, acc, n):
        def part(k):
            for rt in range(k * (D // 8) // n, (k + 1) * (D // 8) // n):
                xc = x_c[8 * rt:8 * rt + 8, :]
                j, r = divmod(rt, D // 8 // len(w_refs))
                p = [w * xc for w in _tiles(w_refs[j], r * width + 2 * b, 2)]
                acc[:] = [u + v for u, v in zip(acc, p)] if rt else p
        return [lambda k=k: part(k) for k in range(n)]

    def q_block(b):
        q = []

        def store():
            for i in range(2):
                q_c[pl.ds(_mult((2 * b + i) * 128, 128), 128), :] = _column(jnp.sum(q[i], axis=0, keepdims=True))
        return x_dot([wq_b.at[0], wq_b.at[1]], H * DH // 128, b, q, 4) + [store]

    def gate_block(b):
        g = []
        x_dot([wg_b], F // 128, b, g, 1)[0]()
        for i in range(2):
            h_c[pl.ds(_mult((2 * b + i) * 128, 128), 8), :] = jnp.broadcast_to(
                jax.nn.silu(jnp.sum(g[i], axis=0, keepdims=True)), (8, 128)) * g_s[1]

    def up_block(b):
        u = []
        x_dot([wu_b], F // 128, b, u, 1)[0]()
        for i in range(2):
            r = _mult((2 * b + i) * 128, 128)
            h_c[pl.ds(r, 128), :] = _column(h_c[pl.ds(r, 8), :][:1] * jnp.sum(u[i], axis=0, keepdims=True))

    def split(a):
        return [a[:, c:c + 128] for c in range(0, D, 128)]

    def proj(half, h, o):
        acc = split(a_s[...])
        for t, w in enumerate(_tiles(wo_b.at[half], h * (DH // 8 * DT), DH // 8 * DT)):
            acc[t % DT] = acc[t % DT] + w * o[8 * (t // DT):8 * (t // DT) + 8]
        a_s[...] = jnp.concatenate(acc, axis=1)

    def down(acc, rt, first, n, quarters=range(4)):
        for j in quarters:
            for t, w in enumerate(_tiles(wd_b.at[j], DT * rt + first, n), first):
                rows = pl.ds(_mult(j * (F // 4) + 8 * (rt + t // DT), 8), 8)
                acc[t % DT] = acc[t % DT] + w * h_c[rows, :]
        return acc

    def attention(h, st):
        head = pl.ds(_mult(h * DH, DH), DH)

        def qk(j):
            q = q_c[head, :]
            for c in range(256 * j, 256 * (j + 1), 128):
                k = k_b[h, :, :, c:c + 128].reshape(DH, 128).astype(f32)
                p_s[:, c:c + 128] = jnp.broadcast_to(jnp.sum(k * q, axis=0, keepdims=True), (8, 128))

        def softmax():
            s = p_s[...] * (DH ** -0.5)
            e = jnp.exp(s - jnp.max(s, axis=-1, keepdims=True))
            p_s[...] = e * (g_s[0][:, :1] / jnp.sum(e, axis=-1, keepdims=True))

        def pv(j):
            for c in range(256 * j, 256 * (j + 1), 128):
                v = v_b[h & (RING - 1), :, :, c:c + 128].reshape(DH, 128).astype(f32)
                part = v * jnp.concatenate([p_s[:, c:c + 128]] * (DH // 8), axis=0)
                st['o'] = st['o'] + part if c else part

        def finish():
            st['o'] = jnp.broadcast_to(jnp.sum(st['o'], axis=-1, keepdims=True), (DH, 128))

        tasks = {s: [lambda j=4 * s + i: qk(j) for i in range(4)] for s in range(4)}
        tasks.update({4 + s: [lambda j=4 * s + i: pv(j) for i in range(4)] for s in range(4)})
        tasks[3].append(softmax)
        tasks[7].append(finish)
        return tasks

    def k_iteration(it, feed, tasks=None, last=False):
        iteration(it, 0, lambda s: [kv(int(last), (it + 1) & (H - 1), s)], feed, tasks or {},
                  GAP_IDLE if tasks is None else GAP_BUSY)

    def q_iteration(it, n=FEED, more=(), tasks=None):
        first = (LEAD + FEED * it) // 2
        k_iteration(it, pieces(parts(wq, wq_b, w_sem.at[it & 1]), first, n // 2) + list(more), tasks)
        pl.when(it > 0)(lambda: landed(wq_b.at[tile_rows(4 * first - 2 * FEED, 2 * FEED)],
                                       w_sem.at[(it - 1) & 1]))

    def gu_feed(it):
        return pieces([(wg, wg_b, w_sem.at[it & 1]), (wu, wu_b, w_sem.at[2 + (it & 1)])],
                      FEED // 2 * (it - IT_GU), FEED // 2)

    def gu_landed(it):
        rows = tile_rows(2 * FEED * (it - IT_GU), 2 * FEED)[1]
        landed(wg_b.at[rows], w_sem.at[it & 1])
        landed(wu_b.at[rows], w_sem.at[2 + (it & 1)])

    small = [pltpu.make_async_copy(x_hbm, x_v, s_sem.at[0]),
             pltpu.make_async_copy(gw_hbm, gw_v, s_sem.at[1]),
             pltpu.make_async_copy(wr_hbm, wr_v, s_sem.at[2])]
    kv(0, 0, 0).start(priority=1)
    for c in small:
        c.start()
    for s in range(1, STEPS):
        kv(0, 0, s).start(priority=1)
    for c in pieces(parts(wq, wq_b, w_sem.at[4]), 0, LEAD // 2):
        c.start(priority=0)
        pl.delay(GAP_BUSY)
    loop(0, IT_GU - 1, q_iteration)
    landed(wq_b.at[tile_rows(0, 2 * LEAD)], w_sem.at[4])

    for c in small:
        c.wait()
    xf = x_v[0].astype(f32)
    gate = jax.nn.sigmoid(jnp.sum(xf * gw_v[...].astype(f32).reshape(1, D), axis=-1, keepdims=True))
    rsel = jax.nn.sigmoid(jnp.sum(xf * wr_v[...].astype(f32).reshape(1, D), axis=-1, keepdims=True))
    g_s[0] = jnp.broadcast_to(gate, (8, 128))
    g_s[1] = jnp.broadcast_to((1.0 - gate) * rsel, (8, 128))
    a_s[...] = jnp.where(jax.lax.broadcasted_iota(jnp.int32, (8, D), 0) == 0, (1.0 - gate) * (xf + xf * 0.0), 0.0)
    for c in range(0, D, 128):
        x_c[c:c + 128, :] = _column(x_v[0, :, c:c + 128].astype(f32))
    d_lead = FEED // 4 * (2 * H - 1 - IT_D)
    q_iteration(IT_GU - 1, FEED - LEAD, pieces(parts(wd, wd_b, w_sem.at[4]), d_lead, LEAD // 4), {})
    k_iteration(IT_GU, gu_feed(IT_GU))
    n = 2 * (FEED - LEAD)
    landed(wq_b.at[tile_rows(wq_b.shape[1] // 8 - n, n)], w_sem.at[(IT_GU - 1) & 1])
    landed(wd_b.at[tile_rows(4 * d_lead, LEAD)], w_sem.at[4])

    def q_projection(it):
        k_iteration(it, gu_feed(it), {2 * j: q_block(4 * (it - IT_GU - 1) + j) for j in range(4)})
        gu_landed(it - 1)

    loop(IT_GU + 1, H - 1, q_projection)
    k_iteration(H - 1, gu_feed(H - 1), last=True)
    gu_landed(H - 2)

    def v_iteration(it, feed, extra, project, nxt=None):
        st = {}
        tasks = attention(it - H, st)
        for s, task in extra:
            tasks[s].append(task)
        if project:
            h = it - IT_PROJ
            tasks[project].append(lambda: proj(0, h, q_c[pl.ds(_mult(h * DH, DH), DH), :]))
            tasks[7].append(lambda: proj(1, h, st['o']))
        else:
            def keep():
                q_c[pl.ds(_mult((it - H) * DH, DH), DH), :] = st['o']
            tasks[7].append(keep)
        iteration(it, 1, nxt or (lambda s: [kv(1, it + 1 - H, s)]), feed, tasks, GAP_BUSY)

    def o_feed(it):
        return pieces(parts(wo, wo_b, w_sem.at[it & 1]), FEED // 2 * (it - IT_O), FEED // 2)

    def o_landed(it):
        landed(wo_b.at[tile_rows(2 * FEED * (it - IT_O), 2 * FEED)], w_sem.at[it & 1])

    def ffn_block(it):
        pl.when(it == IT_O)(lambda: gu_landed(it - 1))
        pl.when(it > IT_O)(lambda: o_landed(it - 1))
        pl.when(it < IT_O + 6)(lambda: gate_block(it - IT_O))
        pl.when(it >= IT_O + 6)(lambda: up_block(it - IT_O - 6))

    def d_feed(it):
        return pieces(parts(wd, wd_b, w_sem.at[it & 1]), FEED // 4 * (it - IT_D), FEED // 4)

    def down_block(it):
        landed(wd_b.at[tile_rows(FEED * (it - IT_D), FEED)], w_sem.at[it & 1])
        a_s[...] = jnp.concatenate(down(split(a_s[...]), FEED // DT * (it - IT_D), 0, FEED), axis=1)

    def d_block(it):
        @pl.when(it == IT_D)
        def _():
            o_landed(it - 1)
            a_s[...] = jnp.concatenate(down(split(a_s[...]), 0, 4 * d_lead, LEAD), axis=1)
        pl.when(it > IT_D)(lambda: down_block(it - 1))

    loop(H, IT_O, lambda it: v_iteration(it, gu_feed(it), [(4, lambda: gu_landed(it - 1))], None))
    loop(IT_O, IT_PROJ, lambda it: v_iteration(it, o_feed(it), [(5, lambda: ffn_block(it))], None))
    loop(IT_PROJ, IT_D, lambda it: v_iteration(it, o_feed(it), [(4, lambda: o_landed(it - 1))], 5))
    loop(IT_D, 2 * H - 1, lambda it: v_iteration(it, d_feed(it), [(4, lambda: d_block(it))], 5))

    it = 2 * H - 1
    first = 4 * d_lead + LEAD
    rest = []
    for j in range(4):
        t = first + LAST
        for n in (TAIL if j == 3 else (sum(TAIL),)):
            rows = pl.ds(8 * t, 8 * n)
            rest.append((j, t, n, pltpu.make_async_copy(wd.at[j, rows], wd_b.at[j, rows], e_sem.at[len(rest)])))
            t += n
        assert 8 * t == wd.shape[1]
    v_iteration(it, pieces(parts(wd, wd_b, w_sem.at[it & 1]), first // 4, LAST // 4),
                [(2, lambda: down_block(it - 1))], 1, lambda s: [] if s else [c[3] for c in rest])

    landed(wd_b.at[tile_rows(first, LAST)], w_sem.at[it & 1])
    acc = down(split(a_s[...]), 0, first, LAST)
    for j, t, n, c in rest:
        c.wait()
        acc = down(acc, 0, t, n, (j,))
    out_ref[0] = jnp.sum(jnp.concatenate(acc, axis=1), axis=0, keepdims=True).astype(bf16)


def _tile_list(w):
    r, c = w.shape
    return w.reshape(r // 8, 8, c // 128, 128).transpose(0, 2, 1, 3).reshape(-1, 128)


@jax.jit
def pallas_gated_mix__sliding_block_cached__moe_arch_mod__decode_kernel(
        A_x, A_k_cache, A_v_cache, A_wq, A_wo, B_x, B_w_r, B_w_gate, B_w_up, B_w_down, gate_w):
    del B_x
    kT = jnp.swapaxes(A_k_cache, 2, 3).reshape(H, DH // 16, 16, SK)
    vT = jnp.swapaxes(A_v_cache, 2, 3).reshape(H, DH // 16, 16, SK)
    wg, wu = _tile_list(B_w_gate), _tile_list(B_w_up)
    wq, wo = _tile_list(A_wq).reshape(2, -1, 128), _tile_list(A_wo).reshape(2, -1, 128)
    wd = _tile_list(B_w_down).reshape(4, -1, 128)
    vmem = pltpu.VMEM
    dma = pltpu.SemaphoreType.DMA
    return pl.pallas_call(
        _kernel,
        out_shape=jax.ShapeDtypeStruct((1, 1, D), bf16),
        in_specs=[pl.BlockSpec(memory_space=pl.ANY)] * 10,
        out_specs=pl.BlockSpec(memory_space=pltpu.VMEM),
        scratch_shapes=[
            vmem((1, 1, D), bf16), vmem((D,), bf16), vmem((D,), bf16),
            vmem(wq.shape, bf16), vmem((H, DH // 16, 16, W), bf16), vmem((RING, DH // 16, 16, W), bf16),
            vmem(wo.shape, bf16), vmem(wg.shape, bf16), vmem(wu.shape, bf16), vmem(wd.shape, bf16),
            vmem((D, 128), f32), vmem((H * DH, 128), f32), vmem((F, 128), f32),
            vmem((8, W), f32), vmem((8, D), f32), vmem((2, 8, 128), f32),
            dma((STEPS,)), dma((5,)), dma((3,)), dma((3 + len(TAIL),)),
        ],
        compiler_params=pltpu.CompilerParams(
            vmem_limit_bytes=100 * 1024 * 1024,
            disable_semaphore_checks=True,
            disable_bounds_checks=True,
        ),
        name="gated_mix_decode",
    )(A_x, kT, vT, wq, wo, B_w_r, wg, wu, wd, gate_w)
```
